```python
import jax
import jax.numpy as jnp

def _softmax(x, axis=-1):
    return jax.nn.softmax(x, axis=axis)
def _gelu(x):
    return jax.nn.gelu(x, approximate=True)
def _silu(x):
    return jax.nn.silu(x)
def _sigmoid(x):
    return jax.nn.sigmoid(x)
def _layernorm(x, axis=-1, eps=1e-5):
    m = jnp.mean(x, axis=axis, keepdims=True)
    v = jnp.var(x, axis=axis, keepdims=True)
    return (x - m) / jnp.sqrt(v + eps)
def _scatter_add(tgt, idx, src, axis=0):
    return tgt.at[idx].add(src)
def _segment_sum(src, seg, n):
    return jax.ops.segment_sum(src, seg, n)
class _Rng:
    def __init__(self, key):
        self._k = key
    def _next(self):
        self._k, sub = jax.random.split(self._k)
        return sub
    def normal(self, shape):
        return jax.random.normal(self._next(), shape, dtype=jnp.bfloat16)
    def randint(self, lo, hi, shape):
        return jax.random.randint(self._next(), shape, lo, hi, dtype=jnp.int32)
    def uniform(self, shape, lo=0.0, hi=1.0):
        return jax.random.uniform(self._next(), shape, jnp.bfloat16, lo, hi)
    def permutation(self, n):
        return jax.random.permutation(self._next(), n)


kernel_name = 'concat_heads__spectral_gfnet__compressed_kv_cla__prompt'

def setup_inputs():
    _rng = _Rng(jax.random.key(int.from_bytes(__import__("os").urandom(4), "little")))
    _w = (lambda a: (lambda t: t.astype(jnp.bfloat16) if jnp.issubdtype(t.dtype, jnp.floating) else t)(jnp.asarray(a)))
    def _A_setup():
        B, S, D = 1, 2048, 448
        Df = D // 2 + 1
        return {
            "x": _w((lambda *s: _rng.normal(s) * 0.05)(B, S, D)),
            "w_r": _w((lambda *s: _rng.normal(s) * 0.05)(S, Df) * 0.02),
            "w_i": _w((lambda *s: _rng.normal(s) * 0.05)(S, Df) * 0.02),
        }
    _A_in = _A_setup()

    def _B_setup():
        B, H, Sq, Sk, D, M = 1, 16, 2048, 2048, 256, 448
        Dc = 4 * D
        return {
            "x": _w((lambda *s: _rng.normal(s) * 0.05)(B, Sq, M)),
            "c_kv": _w((lambda *s: _rng.normal(s) * 0.05)(B, Sk, Dc)),
            "w_q": _w((lambda *s: _rng.normal(s) * 0.05)(M, H, D) * (M ** -0.5)),
            "w_uk": _w((lambda *s: _rng.normal(s) * 0.05)(Dc, H, D) * (Dc ** -0.5)),
            "w_uv": _w((lambda *s: _rng.normal(s) * 0.05)(Dc, H, D) * (Dc ** -0.5)),
            "w_o": _w((lambda *s: _rng.normal(s) * 0.05)(H, D, M) * ((H * D) ** -0.5)),
        }
    _B_in = _B_setup()

    return {
        "A_x": _A_in["x"],
        "A_w_r": _A_in["w_r"],
        "A_w_i": _A_in["w_i"],
        "B_x": _B_in["x"],
        "B_c_kv": _B_in["c_kv"],
        "B_w_q": _B_in["w_q"],
        "B_w_uk": _B_in["w_uk"],
        "B_w_uv": _B_in["w_uv"],
        "B_w_o": _B_in["w_o"],
    }

def reference(A_x, A_w_r, A_w_i, B_x, B_c_kv, B_w_q, B_w_uk, B_w_uv, B_w_o):
    def _A_ref(x, w_r, w_i):
        B, S, D = x.shape
        X = (lambda x, axes=(-2,-1): jnp.fft.rfft2(x.astype(jnp.float32), axes=axes))(x, axes=(-2, -1))
        W = w_r + 1j * w_i
        X = X * W
        y = (lambda x, s, axes=(-2,-1): jnp.fft.irfft2(x, s=s, axes=axes).astype(jnp.bfloat16))(X, (S, D), axes=(-2, -1))
        return y

    def _B_ref(x, c_kv, w_q, w_uk, w_uv, w_o):
        B, Sq, M = x.shape[0], x.shape[1], x.shape[2]
        Sk = c_kv.shape[1]
        H, D = w_q.shape[1], w_q.shape[2]
        q = jnp.einsum("bqm,mhd->bhqd", x, w_q)
        k = jnp.einsum("bkc,chd->bhkd", c_kv, w_uk)
        v = jnp.einsum("bkc,chd->bhkd", c_kv, w_uv)
        scores = jnp.einsum("bhqd,bhkd->bhqk", q, k) * (D ** -0.5)
        off = Sk - Sq
        qi = jnp.arange(Sq)[:, None]
        kj = jnp.arange(Sk)[None, :]
        cmask = kj <= (qi + off)
        scores = jnp.where(cmask[None, None], scores, -1e9)
        p = _softmax(scores, axis=-1)
        ctx = jnp.einsum("bhqk,bhkd->bhqd", p, v)
        return jnp.einsum("bhqd,hdm->bqm", ctx, w_o)

    a = _A_ref(A_x, A_w_r, A_w_i)
    b = _B_ref(B_x, B_c_kv, B_w_q, B_w_uk, B_w_uv, B_w_o)
    return jnp.concatenate([a, b], axis=-1)
```

```python
import functools

import jax
import jax.numpy as jnp
import ml_dtypes
import numpy as np
from jax.experimental import pallas as pl
from jax.experimental.pallas import tpu as pltpu

_BF = ml_dtypes.bfloat16
F32 = jnp.float32
BF16 = jnp.bfloat16
U32 = jnp.uint32

S = 2048
DM = 448
DF = 225
DC = 1024
H = 16
D = 256
BQ = 256

_NT = (((1,), (1,)), ((), ()))
_SCALE = float(np.log2(np.e) / np.sqrt(D))
_C8 = float(np.cos(np.pi / 8))
_S8 = float(np.sin(np.pi / 8))
_R2 = float(np.sqrt(0.5))


def _dft_constants():
    d = np.arange(DM)
    k2 = np.arange(DF)
    ang = 2 * np.pi * (np.outer(d, k2) % DM) / DM
    fd = np.zeros((DM, 512))
    fd[:, 0:DF] = np.cos(ang) / S
    fd[:, 256:256 + DF] = -np.sin(ang) / S
    p = np.arange(128)
    b = np.arange(128)
    gf = np.zeros((16, 256, 128))
    gi = np.zeros((16, 256, 128))
    for q in range(16):
        a = -2 * np.pi * (np.outer(16 * p + q, b) % S) / S
        gf[q, :128] = np.cos(a)
        gf[q, 128:] = np.sin(a)
        gi[q, :128] = np.cos(a).T
        gi[q, 128:] = np.sin(a).T
    cf = np.full(DF, 2.0)
    cf[0] = 1.0
    cf[-1] = 1.0
    fi = np.zeros((512, 512))
    fi[0:DF, :DM] = cf[:, None] * np.cos(ang.T) / DM
    fi[256:256 + DF, :DM] = -cf[:, None] * np.sin(ang.T) / DM
    return tuple(a.astype(np.float32).astype(_BF) for a in (fd, gf, gi, fi))


def _cmul_w(xr, xi, e, sign):
    e = e % 16
    if sign < 0:
        e = (16 - e) % 16
    q, r = divmod(e, 4)
    if r == 0:
        yr, yi = xr, xi
    elif r == 2:
        yr, yi = (xr - xi) * _R2, (xr + xi) * _R2
    elif r == 1:
        yr, yi = xr * _C8 - xi * _S8, xr * _S8 + xi * _C8
    else:
        yr, yi = xr * _S8 - xi * _C8, xr * _C8 + xi * _S8
    return yr, yi, q


def _addsub(a, b, extra=1):
    (x, sx), (y, sy) = a, b
    sy = sy * extra
    if sx > 0 and sy > 0:
        return x + y, 1
    if sx > 0 and sy < 0:
        return x - y, 1
    if sx < 0 and sy > 0:
        return y - x, 1
    return x + y, -1


def _dft4(xs, sign):
    def norm(x):
        r, i, rot = x
        rot %= 4
        if rot == 0:
            return (r, 1), (i, 1)
        if rot == 1:
            return (i, -1), (r, 1)
        if rot == 2:
            return (r, -1), (i, -1)
        return (i, 1), (r, -1)

    x = [norm(t) for t in xs]
    t0 = (_addsub(x[0][0], x[2][0]), _addsub(x[0][1], x[2][1]))
    t1 = (_addsub(x[0][0], x[2][0], -1), _addsub(x[0][1], x[2][1], -1))
    t2 = (_addsub(x[1][0], x[3][0]), _addsub(x[1][1], x[3][1]))
    t3 = (_addsub(x[1][0], x[3][0], -1), _addsub(x[1][1], x[3][1], -1))
    x0 = (_addsub(t0[0], t2[0]), _addsub(t0[1], t2[1]))
    x2 = (_addsub(t0[0], t2[0], -1), _addsub(t0[1], t2[1], -1))
    x1 = (_addsub(t1[0], t3[1], -sign), _addsub(t1[1], t3[0], sign))
    x3 = (_addsub(t1[0], t3[1], sign), _addsub(t1[1], t3[0], -sign))
    return [x0, x1, x2, x3]


def _fin(v):
    x, s = v
    return x if s > 0 else -x


def _dft16(xr, xi, sign):
    u = [[None] * 4 for _ in range(4)]
    for a0 in range(4):
        o = _dft4([(xr[a0 + 4 * a1], xi[a0 + 4 * a1], 0) for a1 in range(4)], sign)
        for q0 in range(4):
            (r, sr), (i, si) = o[q0]
            assert sr > 0 and si > 0
            u[a0][q0] = _cmul_w(r, i, a0 * q0, sign)
    yr = [None] * 16
    yi = [None] * 16
    for q0 in range(4):
        o = _dft4([u[a0][q0] for a0 in range(4)], sign)
        for q1 in range(4):
            yr[q0 + 4 * q1] = _fin(o[q1][0])
            yi[q0 + 4 * q1] = _fin(o[q1][1])
    return yr, yi


def _lo(u):
    return pltpu.bitcast(u << 16, F32)


def _hi(u):
    return pltpu.bitcast(u & jnp.uint32(0xFFFF0000), F32)


def _part_a(xat_ref, wt_ref, fd_ref, gf_ref, gi_ref, fi_ref, y_out_ref,
            wait_x, wait_w, wait_g, wait_fi, y_ref, t_ref, z_ref, wn_ref):
    rc = 16
    wait_x()
    for i in range(8):
        xa = xat_ref[:, 256 * i:256 * i + 256].T
        y_ref[256 * i:256 * i + 256, :] = jnp.dot(xa, fd_ref[...], preferred_element_type=F32)
    wait_w()
    for ri in range(2):
        for a in range(16):
            wn_ref[2 * ri, 128 * a:128 * a + 128, :] = wt_ref[ri, 0:128, 128 * a:128 * a + 128].T
            wn_ref[2 * ri + 1, 128 * a:128 * a + 128, 0:DF - 128] = (
                wt_ref[ri, 128:DF, 128 * a:128 * a + 128].T)
    for t in range(2):
        for r in range(0, 128, rc):
            xr = [y_ref[128 * a + r:128 * a + r + rc, 128 * t:128 * t + 128] for a in range(16)]
            xi = [y_ref[128 * a + r:128 * a + r + rc, 256 + 128 * t:384 + 128 * t] for a in range(16)]
            yr, yi = _dft16(xr, xi, -1)
            for q in range(16):
                t_ref[q, r:r + rc, 128 * t:128 * t + 128] = yr[q].astype(BF16)
                t_ref[q, r:r + rc, 256 + 128 * t:384 + 128 * t] = yi[q].astype(BF16)
    wait_g()
    lane = jax.lax.broadcasted_iota(jnp.int32, (128, 128), 1)
    wn32 = wn_ref.bitcast(U32)
    for j in range(8):
        wrs = [wn32[t, pl.ds(j, 128, stride=8), :] for t in range(2)]
        wis = [wn32[2 + t, pl.ds(j, 128, stride=8), :] for t in range(2)]
        for e in range(2):
            q = 2 * j + e
            m = jnp.dot(gf_ref[q], t_ref[q], preferred_element_type=F32)
            unp = _lo if e == 0 else _hi
            for t in range(2):
                xr = m[0:128, 128 * t:128 * t + 128] - m[128:256, 256 + 128 * t:384 + 128 * t]
                xi = m[128:256, 128 * t:128 * t + 128] + m[0:128, 256 + 128 * t:384 + 128 * t]
                wr = unp(wrs[t])
                wi = unp(wis[t])
                zr = xr * wr - xi * wi
                zi = xr * wi + xi * wr
                if t == 1:
                    zr = jnp.where(lane < DF - 128, zr, 0.0)
                    zi = jnp.where(lane < DF - 128, zi, 0.0)
                z_ref[q, :, 128 * t:128 * t + 128] = zr.astype(BF16)
                z_ref[q, :, 256 + 128 * t:384 + 128 * t] = zi.astype(BF16)
    for q in range(16):
        m = jnp.dot(gi_ref[q], z_ref[q], preferred_element_type=F32)
        y_ref[128 * q:128 * q + 128, 0:256] = m[0:128, 0:256] + m[128:256, 256:512]
        y_ref[128 * q:128 * q + 128, 256:512] = m[0:128, 256:512] - m[128:256, 0:256]
    for t in range(2):
        for r in range(0, 128, rc):
            xr = [y_ref[128 * q + r:128 * q + r + rc, 128 * t:128 * t + 128] for q in range(16)]
            xi = [y_ref[128 * q + r:128 * q + r + rc, 256 + 128 * t:384 + 128 * t] for q in range(16)]
            yr, yi = _dft16(xr, xi, 1)
            for a in range(16):
                t_ref[a, r:r + rc, 128 * t:128 * t + 128] = yr[a].astype(BF16)
                t_ref[a, r:r + rc, 256 + 128 * t:384 + 128 * t] = yi[a].astype(BF16)
    wait_fi()
    for a in range(16):
        y_out_ref[128 * a:128 * a + 128, :] = jnp.dot(
            t_ref[a], fi_ref[...], preferred_element_type=F32).astype(BF16)


def _relayout_pair(raw_k, raw_v, raw_q, wkv_ref, wq_ref):
    for e, unp in enumerate((_lo, _hi)):
        for r in range(0, DC, 256):
            wkv_ref[e, r:r + 256, 0:256] = unp(raw_k[r:r + 256, :]).astype(BF16)
            wkv_ref[e, r:r + 256, 256:512] = unp(raw_v[r:r + 256, :]).astype(BF16)
        for r in range(0, DM, 224):
            wq_ref[e, r:r + 224, :] = unp(raw_q[r:r + 224, :]).astype(BF16)


def _proj_chunk(i, c_ref, x_ref, wkv, wq, k_ref, v_ref, q_ref):
    r0 = BQ * i
    kv = jnp.dot(c_ref[r0:r0 + BQ, :], wkv[...], preferred_element_type=F32)
    k_ref[r0:r0 + BQ, :] = kv[:, 0:256].astype(BF16)
    v_ref[r0:r0 + BQ, :] = kv[:, 256:512].astype(BF16)
    q = jnp.dot(x_ref[r0:r0 + BQ, :], wq[...], preferred_element_type=F32)
    q_ref[r0:r0 + BQ, :] = (q * _SCALE).astype(BF16)


def _qk(i, q_ref, k_ref):
    r0 = BQ * i
    hb = BQ // 2
    row = jax.lax.broadcasted_iota(jnp.int32, (hb, hb), 0)
    col = jax.lax.broadcasted_iota(jnp.int32, (hb, hb), 1)
    tri = col <= row
    q = q_ref[r0:r0 + BQ, :]
    s_off = None
    if i > 0:
        s_off = jax.lax.dot_general(q, k_ref[0:r0, :], _NT, preferred_element_type=F32)
    s_d1 = jax.lax.dot_general(q[0:hb], k_ref[r0:r0 + hb, :], _NT, preferred_element_type=F32)
    s_d2 = jax.lax.dot_general(q[hb:BQ], k_ref[r0:r0 + BQ, :], _NT, preferred_element_type=F32)
    s_d1 = jnp.where(tri, s_d1, -1e30)
    s_d2a = s_d2[:, 0:hb]
    s_d2b = jnp.where(tri, s_d2[:, hb:BQ], -1e30)
    return s_off, s_d1, s_d2a, s_d2b


def _rowmax(x):
    return jnp.max(x, axis=1, keepdims=True)


def _rowsum(x):
    return jnp.sum(x, axis=1, keepdims=True)


def _pv(i, s, v_ref, ctx_ref, col0):
    r0 = BQ * i
    hb = BQ // 2
    s_off, s_d1, s_d2a, s_d2b = s
    m1 = _rowmax(s_d1)
    m2 = _rowmax(jnp.maximum(s_d2a, s_d2b))
    if s_off is not None:
        mo = _rowmax(s_off)
        m1 = jnp.maximum(m1, mo[0:hb])
        m2 = jnp.maximum(m2, mo[hb:BQ])
    p1 = jnp.exp2(s_d1 - m1)
    p2a = jnp.exp2(s_d2a - m2)
    p2b = jnp.exp2(s_d2b - m2)
    l1 = _rowsum(p1)
    l2 = _rowsum(p2a + p2b)
    o1 = jnp.dot(p1.astype(BF16), v_ref[r0:r0 + hb, :], preferred_element_type=F32)
    p2 = jnp.concatenate([p2a.astype(BF16), p2b.astype(BF16)], axis=1)
    o2 = jnp.dot(p2, v_ref[r0:r0 + BQ, :], preferred_element_type=F32)
    if s_off is not None:
        m = jnp.concatenate([m1, m2], axis=0)
        po = jnp.exp2(s_off - m)
        lo = _rowsum(po)
        oo = jnp.dot(po.astype(BF16), v_ref[0:r0, :], preferred_element_type=F32)
        l1 = l1 + lo[0:hb]
        l2 = l2 + lo[hb:BQ]
        o1 = o1 + oo[0:hb]
        o2 = o2 + oo[hb:BQ]
    ctx_ref[r0:r0 + hb, pl.ds(col0, D)] = (o1 * (1.0 / l1)).astype(BF16)
    ctx_ref[r0 + hb:r0 + BQ, pl.ds(col0, D)] = (o2 * (1.0 / l2)).astype(BF16)


def _attn_head(q_ref, k_ref, v_ref, ctx_ref, col0, filler):
    for i in range(S // BQ):
        s = _qk(i, q_ref, k_ref)
        if filler is not None:
            filler(i)
        _pv(i, s, v_ref, ctx_ref, col0)


def _kernel(xat_hbm, wrt_hbm, wit_hbm, xbt_hbm, c_hbm, wq_hbm, wk_hbm, wv_hbm, wot_hbm,
            fd_hbm, gf_hbm, gi_hbm, fi_hbm, out_hbm,
            xbt_ref, xb_ref, c_ref, rawk, rawv, rawq, wkv_ref, wqh_ref,
            k_ref, v_ref, q_ref, ctx_ref, wot_ref, y_out_ref, sem, osem):
    wq32 = wq_hbm.bitcast(U32)
    wk32 = wk_hbm.bitcast(U32)
    wv32 = wv_hbm.bitcast(U32)

    def pair_copies(j, slot):
        return [
            pltpu.make_async_copy(wk32.at[:, j, :], rawk.at[slot], sem.at[16 + 3 * slot]),
            pltpu.make_async_copy(wv32.at[:, j, :], rawv.at[slot], sem.at[17 + 3 * slot]),
            pltpu.make_async_copy(wq32.at[:, j, :], rawq.at[slot], sem.at[18 + 3 * slot]),
        ]

    def phase_a(xat_ref, wt_ref, fd_ref, gf_ref, gi_ref, fi_ref, y_ref, t_ref, z_ref, wn_ref):
        cp_x = pltpu.make_async_copy(xat_hbm, xat_ref, sem.at[0])
        cp_fd = pltpu.make_async_copy(fd_hbm, fd_ref, sem.at[1])
        cp_wr = pltpu.make_async_copy(wrt_hbm, wt_ref.at[0], sem.at[2])
        cp_wi = pltpu.make_async_copy(wit_hbm, wt_ref.at[1], sem.at[3])
        cp_gf = pltpu.make_async_copy(gf_hbm, gf_ref, sem.at[4])
        cp_gi = pltpu.make_async_copy(gi_hbm, gi_ref, sem.at[5])
        cp_fi = pltpu.make_async_copy(fi_hbm, fi_ref, sem.at[6])
        cp_xb = pltpu.make_async_copy(xbt_hbm, xbt_ref, sem.at[7])
        cp_c = pltpu.make_async_copy(c_hbm, c_ref, sem.at[8])
        for cp in (cp_x, cp_fd, cp_wr, cp_wi, cp_gf, cp_gi, cp_fi, cp_xb, cp_c):
            cp.start()
        for cp in pair_copies(0, 0):
            cp.start()
        for cp in pair_copies(1, 1):
            cp.start()

        def wait_x():
            cp_x.wait()
            cp_fd.wait()

        def wait_w():
            cp_wr.wait()
            cp_wi.wait()

        def wait_g():
            cp_gf.wait()
            cp_gi.wait()

        def wait_fi():
            cp_fi.wait()
            cp_xb.wait()
            for i in range(8):
                xb_ref[256 * i:256 * i + 256, :] = xbt_ref[:, 256 * i:256 * i + 256].T

        _part_a(xat_ref, wt_ref, fd_ref, gf_ref, gi_ref, fi_ref, y_out_ref,
                wait_x, wait_w, wait_g, wait_fi, y_ref, t_ref, z_ref, wn_ref)
        cp_c.wait()

    pl.run_scoped(
        phase_a,
        pltpu.VMEM((DM, S), BF16),
        pltpu.VMEM((2, DF, S), BF16),
        pltpu.VMEM((DM, 512), BF16),
        pltpu.VMEM((16, 256, 128), BF16),
        pltpu.VMEM((16, 256, 128), BF16),
        pltpu.VMEM((512, 512), BF16),
        pltpu.VMEM((S, 512), F32),
        pltpu.VMEM((16, 128, 512), BF16),
        pltpu.VMEM((16, 128, 512), BF16),
        pltpu.VMEM((4, S, 128), BF16),
    )

    cp_y = pltpu.make_async_copy(y_out_ref.at[:, pl.ds(0, 384)], out_hbm.at[:, pl.ds(0, 384)], osem.at[0])
    cp_y.start()

    wot_ref[0:64, :] = jnp.zeros((64, H * D), BF16)
    cp_wo = [pltpu.make_async_copy(wot_hbm.at[h], wot_ref.at[pl.ds(64, DM), pl.ds(D * h, D)], sem.at[22 + h])
             for h in range(H)]

    def proj_filler(e, slot):
        return lambda i: _proj_chunk(i, c_ref, xb_ref, wkv_ref.at[e], wqh_ref.at[e],
                                     k_ref.at[slot], v_ref.at[slot], q_ref.at[slot])

    def wait_relayout(j, slot):
        for cp in pair_copies(j, slot):
            cp.wait()
        _relayout_pair(rawk.at[slot], rawv.at[slot], rawq.at[slot], wkv_ref, wqh_ref)

    wait_relayout(0, 0)
    for i in range(S // BQ):
        proj_filler(0, 0)(i)

    def pair_body(j, slot, last):
        col = pl.multiple_of(j * (2 * D), 2 * D)
        _attn_head(q_ref.at[0], k_ref.at[0], v_ref.at[0], ctx_ref, col, proj_filler(1, 1))
        if not last:
            wait_relayout(j + 1, 1 - slot)

            @pl.when(j + 2 < H // 2)
            def _():
                for cp in pair_copies(j + 2, slot):
                    cp.start()
        _attn_head(q_ref.at[1], k_ref.at[1], v_ref.at[1], ctx_ref, col + D,
                   None if last else proj_filler(0, 0))

    def two_pairs(jj, carry):
        pair_body(2 * jj, 0, False)

        @pl.when(jj == 0)
        def _():
            for cp in cp_wo:
                cp.start()
        pair_body(2 * jj + 1, 1, False)
        return carry

    jax.lax.fori_loop(0, 3, two_pairs, 0)
    pair_body(6, 0, False)
    pair_body(7, 1, True)

    for cp in cp_wo:
        cp.wait()
    cp_y.wait()
    rb = 512
    out_cps = []
    for i in range(S // rb):
        b = jax.lax.dot_general(ctx_ref[rb * i:rb * i + rb, :], wot_ref[...], _NT, preferred_element_type=F32)
        first = b[:, 0:128] + y_out_ref[rb * i:rb * i + rb, 384:512].astype(F32)
        y_out_ref[rb * i:rb * i + rb, 0:128] = first.astype(BF16)
        y_out_ref[rb * i:rb * i + rb, 128:512] = b[:, 128:512].astype(BF16)
        cp = pltpu.make_async_copy(y_out_ref.at[pl.ds(rb * i, rb), :],
                                   out_hbm.at[pl.ds(rb * i, rb), pl.ds(384, 512)], osem.at[1 + i])
        cp.start()
        out_cps.append(cp)
    for cp in out_cps:
        cp.wait()


def _run(A_x, A_w_r, A_w_i, B_x, B_c_kv, B_w_q, B_w_uk, B_w_uv, B_w_o):
    fd, gf, gi, fi = _dft_constants()
    any_spec = pl.BlockSpec(memory_space=pl.ANY)
    out = pl.pallas_call(
        _kernel,
        out_shape=jax.ShapeDtypeStruct((S, 2 * DM), BF16),
        in_specs=[any_spec] * 13,
        out_specs=any_spec,
        scratch_shapes=[
            pltpu.VMEM((DM, S), BF16),
            pltpu.VMEM((S, DM), BF16),
            pltpu.VMEM((S, DC), BF16),
            pltpu.VMEM((2, DC, D), U32),
            pltpu.VMEM((2, DC, D), U32),
            pltpu.VMEM((2, DM, D), U32),
            pltpu.VMEM((2, DC, 2 * D), BF16),
            pltpu.VMEM((2, DM, D), BF16),
            pltpu.VMEM((2, S, D), BF16),
            pltpu.VMEM((2, S, D), BF16),
            pltpu.VMEM((2, S, D), BF16),
            pltpu.VMEM((S, H * D), BF16),
            pltpu.VMEM((512, H * D), BF16),
            pltpu.VMEM((S, 512), BF16),
            pltpu.SemaphoreType.DMA((40,)),
            pltpu.SemaphoreType.DMA((8,)),
        ],
        compiler_params=pltpu.CompilerParams(vmem_limit_bytes=110 * 1024 * 1024),
    )(A_x[0].T, A_w_r.T, A_w_i.T, B_x[0].T, B_c_kv[0], B_w_q, B_w_uk, B_w_uv,
      jnp.swapaxes(B_w_o, 1, 2), fd, gf, gi, fi)
    return out[None]


@jax.jit
def pallas_concat_heads__spectral_gfnet__compressed_kv_cla__prompt_kernel(
    A_x: jax.Array,
    A_w_r: jax.Array,
    A_w_i: jax.Array,
    B_x: jax.Array,
    B_c_kv: jax.Array,
    B_w_q: jax.Array,
    B_w_uk: jax.Array,
    B_w_uv: jax.Array,
    B_w_o: jax.Array,
):
    return _run(A_x, A_w_r, A_w_i, B_x, B_c_kv, B_w_q, B_w_uk, B_w_uv, B_w_o)
```

```python
import functools

import jax
import jax.numpy as jnp
import ml_dtypes
import numpy as np
from jax.experimental import pallas as pl
from jax.experimental.pallas import tpu as pltpu

_BF = ml_dtypes.bfloat16
F32 = jnp.float32
BF16 = jnp.bfloat16
U32 = jnp.uint32

S = 2048
DM = 448
DF = 225
DC = 1024
H = 16
D = 256
BQ = 256

_NT = (((1,), (1,)), ((), ()))
_SCALE = float(np.log2(np.e) / np.sqrt(D))
_C8 = float(np.cos(np.pi / 8))
_S8 = float(np.sin(np.pi / 8))
_R2 = float(np.sqrt(0.5))


def _dft_constants():
    d = np.arange(DM)
    k2 = np.arange(DF)
    ang = 2 * np.pi * (np.outer(d, k2) % DM) / DM
    fd = np.zeros((DM, 512))
    fd[:, 0:DF] = np.cos(ang) / S
    fd[:, 256:256 + DF] = -np.sin(ang) / S
    p = np.arange(128)
    b = np.arange(128)
    gf = np.zeros((16, 256, 128))
    gi = np.zeros((16, 256, 128))
    for q in range(16):
        a = -2 * np.pi * (np.outer(16 * p + q, b) % S) / S
        gf[q, :128] = np.cos(a)
        gf[q, 128:] = np.sin(a)
        gi[q, :128] = np.cos(a).T
        gi[q, 128:] = np.sin(a).T
    cf = np.full(DF, 2.0)
    cf[0] = 1.0
    cf[-1] = 1.0
    fi = np.zeros((512, 512))
    fi[0:DF, :DM] = cf[:, None] * np.cos(ang.T) / DM
    fi[256:256 + DF, :DM] = -cf[:, None] * np.sin(ang.T) / DM
    return tuple(a.astype(np.float32).astype(_BF) for a in (fd, gf, gi, fi))


def _cmul_w(xr, xi, e, sign):
    e = e % 16
    if sign < 0:
        e = (16 - e) % 16
    q, r = divmod(e, 4)
    if r == 0:
        yr, yi = xr, xi
    elif r == 2:
        yr, yi = (xr - xi) * _R2, (xr + xi) * _R2
    elif r == 1:
        yr, yi = xr * _C8 - xi * _S8, xr * _S8 + xi * _C8
    else:
        yr, yi = xr * _S8 - xi * _C8, xr * _C8 + xi * _S8
    return yr, yi, q


def _addsub(a, b, extra=1):
    (x, sx), (y, sy) = a, b
    sy = sy * extra
    if sx > 0 and sy > 0:
        return x + y, 1
    if sx > 0 and sy < 0:
        return x - y, 1
    if sx < 0 and sy > 0:
        return y - x, 1
    return x + y, -1


def _dft4(xs, sign):
    def norm(x):
        r, i, rot = x
        rot %= 4
        if rot == 0:
            return (r, 1), (i, 1)
        if rot == 1:
            return (i, -1), (r, 1)
        if rot == 2:
            return (r, -1), (i, -1)
        return (i, 1), (r, -1)

    x = [norm(t) for t in xs]
    t0 = (_addsub(x[0][0], x[2][0]), _addsub(x[0][1], x[2][1]))
    t1 = (_addsub(x[0][0], x[2][0], -1), _addsub(x[0][1], x[2][1], -1))
    t2 = (_addsub(x[1][0], x[3][0]), _addsub(x[1][1], x[3][1]))
    t3 = (_addsub(x[1][0], x[3][0], -1), _addsub(x[1][1], x[3][1], -1))
    x0 = (_addsub(t0[0], t2[0]), _addsub(t0[1], t2[1]))
    x2 = (_addsub(t0[0], t2[0], -1), _addsub(t0[1], t2[1], -1))
    x1 = (_addsub(t1[0], t3[1], -sign), _addsub(t1[1], t3[0], sign))
    x3 = (_addsub(t1[0], t3[1], sign), _addsub(t1[1], t3[0], -sign))
    return [x0, x1, x2, x3]


def _fin(v):
    x, s = v
    return x if s > 0 else -x


def _dft16(xr, xi, sign):
    u = [[None] * 4 for _ in range(4)]
    for a0 in range(4):
        o = _dft4([(xr[a0 + 4 * a1], xi[a0 + 4 * a1], 0) for a1 in range(4)], sign)
        for q0 in range(4):
            (r, sr), (i, si) = o[q0]
            assert sr > 0 and si > 0
            u[a0][q0] = _cmul_w(r, i, a0 * q0, sign)
    yr = [None] * 16
    yi = [None] * 16
    for q0 in range(4):
        o = _dft4([u[a0][q0] for a0 in range(4)], sign)
        for q1 in range(4):
            yr[q0 + 4 * q1] = _fin(o[q1][0])
            yi[q0 + 4 * q1] = _fin(o[q1][1])
    return yr, yi


def _lo(u):
    return pltpu.bitcast(u << 16, F32)


def _hi(u):
    return pltpu.bitcast(u & jnp.uint32(0xFFFF0000), F32)


_RC = 16


def _a_feature_dft(i, xat_ref, fd_ref, y_ref):
    xa = xat_ref[:, 256 * i:256 * i + 256].T
    y_ref[256 * i:256 * i + 256, :] = jnp.dot(xa, fd_ref[...], preferred_element_type=F32)


def _a_dft16(r, sign, y_ref, t_ref):
    r = r * _RC
    for t in range(2):
        xr = [y_ref[128 * a + r:128 * a + r + _RC, 128 * t:128 * t + 128] for a in range(16)]
        xi = [y_ref[128 * a + r:128 * a + r + _RC, 256 + 128 * t:384 + 128 * t] for a in range(16)]
        yr, yi = _dft16(xr, xi, sign)
        for q in range(16):
            t_ref[q, r:r + _RC, 128 * t:128 * t + 128] = yr[q].astype(BF16)
            t_ref[q, r:r + _RC, 256 + 128 * t:384 + 128 * t] = yi[q].astype(BF16)


def _a_w_transpose(a, wt_ref, wn_ref):
    for ri in range(2):
        wn_ref[2 * ri, 128 * a:128 * a + 128, :] = wt_ref[ri, 0:128, 128 * a:128 * a + 128].T
        wn_ref[2 * ri + 1, 128 * a:128 * a + 128, 0:DF - 128] = (
            wt_ref[ri, 128:DF, 128 * a:128 * a + 128].T)


def _a_fwd_gate(q, gf_ref, t_ref, wn_ref, z_ref):
    lane = jax.lax.broadcasted_iota(jnp.int32, (128, 128), 1)
    wn32 = wn_ref.bitcast(U32)
    j, e = divmod(q, 2)
    unp = _lo if e == 0 else _hi
    m = jnp.dot(gf_ref[q], t_ref[q], preferred_element_type=F32)
    for t in range(2):
        xr = m[0:128, 128 * t:128 * t + 128] - m[128:256, 256 + 128 * t:384 + 128 * t]
        xi = m[128:256, 128 * t:128 * t + 128] + m[0:128, 256 + 128 * t:384 + 128 * t]
        wr = unp(wn32[t, pl.ds(j, 128, stride=8), :])
        wi = unp(wn32[2 + t, pl.ds(j, 128, stride=8), :])
        zr = xr * wr - xi * wi
        zi = xr * wi + xi * wr
        if t == 1:
            zr = jnp.where(lane < DF - 128, zr, 0.0)
            zi = jnp.where(lane < DF - 128, zi, 0.0)
        z_ref[q, :, 128 * t:128 * t + 128] = zr.astype(BF16)
        z_ref[q, :, 256 + 128 * t:384 + 128 * t] = zi.astype(BF16)


def _a_inv(q, gi_ref, z_ref, y_ref):
    m = jnp.dot(gi_ref[q], z_ref[q], preferred_element_type=F32)
    y_ref[128 * q:128 * q + 128, 0:256] = m[0:128, 0:256] + m[128:256, 256:512]
    y_ref[128 * q:128 * q + 128, 256:512] = m[0:128, 256:512] - m[128:256, 0:256]


def _a_feature_idft(a, t_ref, fi_ref, y_out_ref):
    y_out_ref[128 * a:128 * a + 128, :] = jnp.dot(
        t_ref[a], fi_ref[...], preferred_element_type=F32).astype(BF16)


def _relayout_piece(i, unp, raw_k, raw_v, raw_q, wb_ref, wq_ref):
    r = 64 * i
    hc = DC // 2
    b11 = unp(raw_k[pl.ds(r, 64), :])
    b21 = unp(raw_k[pl.ds(hc + r, 64), :])
    b12 = unp(raw_v[pl.ds(r, 64), :])
    b22 = unp(raw_v[pl.ds(hc + r, 64), :])
    for j, b in enumerate(_strassen_rhs(b11, b12, b21, b22)):
        wb_ref[j, pl.ds(r, 64), :] = b.astype(BF16)
    if wq_ref is not None:
        _relayout_q(i, unp, raw_q, wq_ref)


def _strassen_rhs(b11, b12, b21, b22):
    return (b11 + b22, b11, b12 - b22, b21 - b11, b22, b11 + b12, b21 + b22)


def _relayout_q(i, unp, raw_q, wq_ref):
    hm = DM // 2
    if i < 7:
        r = 32 * i
        top = unp(raw_q[r:r + 32, :])
        bot = unp(raw_q[hm + r:hm + r + 32, :])
        for j, b in enumerate(_strassen_rhs(top[:, 0:128], top[:, 128:256], bot[:, 0:128], bot[:, 128:256])):
            wq_ref[j, r:r + 32, :] = b.astype(BF16)


def _strassen_lhs(i, c_ref, ca_ref):
    t0 = 128 * i
    b0 = S // 2 + 128 * i
    hc = DC // 2
    a11 = c_ref[pl.ds(t0, 128), 0:hc].astype(F32)
    a12 = c_ref[pl.ds(t0, 128), hc:DC].astype(F32)
    a21 = c_ref[pl.ds(b0, 128), 0:hc].astype(F32)
    a22 = c_ref[pl.ds(b0, 128), hc:DC].astype(F32)
    for j, a in enumerate((a11 + a22, a21 + a22, a11 + a12, a21 - a11, a12 - a22)):
        ca_ref[j, pl.ds(t0, 128), :] = a.astype(BF16)


def _strassen_products(m, emit):
    m3 = m(3)
    m5 = m(5)
    emit(12, m3 + m5)
    c22 = m3 + m(6)
    m2 = m(2)
    c22 = c22 - m2
    m4 = m(4)
    emit(21, m2 + m4)
    c11 = m4 - m5
    m1 = m(1)
    emit(22, c22 + m1)
    c11 = c11 + m1
    emit(11, c11 + m(7))


def _kv_chunk(i, c_ref, ca_ref, wb, k_ref, v_ref):
    top = pl.ds(128 * i, 128)
    bot = pl.ds(S // 2 + 128 * i, 128)
    hc = DC // 2
    lhs = [ca_ref[0, top, :], ca_ref[1, top, :], c_ref[top, 0:hc], c_ref[bot, hc:DC],
           ca_ref[2, top, :], ca_ref[3, top, :], ca_ref[4, top, :]]

    def emit(b, val):
        (k_ref if b % 10 == 1 else v_ref)[top if b < 20 else bot, :] = val.astype(BF16)

    _strassen_products(lambda j: jnp.dot(lhs[j - 1], wb[j - 1], preferred_element_type=F32), emit)


def _q_chunk(i, xa_ref, wq, q_ref):
    top = pl.ds(128 * i, 128)
    bot = pl.ds(S // 2 + 128 * i, 128)

    def emit(b, val):
        cols = pl.ds(0 if b % 10 == 1 else 128, 128)
        q_ref[top if b < 20 else bot, cols] = (val * _SCALE).astype(BF16)

    _strassen_products(
        lambda j: jnp.dot(xa_ref[j - 1, top, :], wq[j - 1], preferred_element_type=F32), emit)


def _x_lhs(i, xt_ref, xa_ref):
    hm = DM // 2
    r = 256 * i
    a11 = xt_ref[0:hm, r:r + 256].T.astype(F32)
    a12 = xt_ref[hm:DM, r:r + 256].T.astype(F32)
    a21 = xt_ref[0:hm, S // 2 + r:S // 2 + r + 256].T.astype(F32)
    a22 = xt_ref[hm:DM, S // 2 + r:S // 2 + r + 256].T.astype(F32)
    for j, a in enumerate((a11 + a22, a21 + a22, a11, a22, a11 + a12, a21 - a11, a12 - a22)):
        xa_ref[j, r:r + 256, :] = a.astype(BF16)


def _qk(i, q_ref, k_ref):
    r0 = BQ * i
    hb = BQ // 2
    row = jax.lax.broadcasted_iota(jnp.int32, (hb, hb), 0)
    col = jax.lax.broadcasted_iota(jnp.int32, (hb, hb), 1)
    tri = col <= row
    q = q_ref[r0:r0 + BQ, :]
    s_off = None
    if i > 0:
        s_off = jax.lax.dot_general(q, k_ref[0:r0, :], _NT, preferred_element_type=F32)
    s_d1 = jax.lax.dot_general(q[0:hb], k_ref[r0:r0 + hb, :], _NT, preferred_element_type=F32)
    s_d2 = jax.lax.dot_general(q[hb:BQ], k_ref[r0:r0 + BQ, :], _NT, preferred_element_type=F32)
    s_d1 = jnp.where(tri, s_d1, -1e30)
    s_d2a = s_d2[:, 0:hb]
    s_d2b = jnp.where(tri, s_d2[:, hb:BQ], -1e30)
    return s_off, s_d1, s_d2a, s_d2b


def _rowmax(x):
    return jnp.max(x, axis=1, keepdims=True)


def _rowsum(x):
    return jnp.sum(x, axis=1, keepdims=True)


def _pv(i, s, v_ref, ctx_ref, cols):
    r0 = BQ * i
    hb = BQ // 2
    s_off, s_d1, s_d2a, s_d2b = s
    m1 = _rowmax(s_d1)
    m2 = _rowmax(jnp.maximum(s_d2a, s_d2b))
    if s_off is not None:
        mo = _rowmax(s_off)
        m1 = jnp.maximum(m1, mo[0:hb])
        m2 = jnp.maximum(m2, mo[hb:BQ])
    p1 = jnp.exp2(s_d1 - m1)
    p2a = jnp.exp2(s_d2a - m2)
    p2b = jnp.exp2(s_d2b - m2)
    l1 = _rowsum(p1)
    l2 = _rowsum(p2a + p2b)
    o1 = jnp.dot(p1.astype(BF16), v_ref[r0:r0 + hb, :], preferred_element_type=F32)
    p2 = jnp.concatenate([p2a.astype(BF16), p2b.astype(BF16)], axis=1)
    o2 = jnp.dot(p2, v_ref[r0:r0 + BQ, :], preferred_element_type=F32)
    if s_off is not None:
        m = jnp.concatenate([m1, m2], axis=0)
        po = jnp.exp2(s_off - m)
        lo = _rowsum(po)
        oo = jnp.dot(po.astype(BF16), v_ref[0:r0, :], preferred_element_type=F32)
        l1 = l1 + lo[0:hb]
        l2 = l2 + lo[hb:BQ]
        o1 = o1 + oo[0:hb]
        o2 = o2 + oo[hb:BQ]
    ctx_ref[r0:r0 + hb, cols] = (o1 * (1.0 / l1)).astype(BF16)
    ctx_ref[r0 + hb:r0 + BQ, cols] = (o2 * (1.0 / l2)).astype(BF16)


def _attn_head(q_ref, k_ref, v_ref, ctx_ref, h, filler):
    cols = pl.ds(h * D if isinstance(h, int) else pl.multiple_of(h * D, D), D)
    for i in range(S // BQ):
        s = _qk(i, q_ref, k_ref)
        filler(i)
        _pv(i, s, v_ref, ctx_ref, cols)


def _out_lhs(wot_ref, wa_ref):
    hm = DM // 2
    hk = H * D // 2
    for c in range(0, hk, 512):
        a11 = wot_ref[0:hm, c:c + 512].astype(F32)
        a12 = wot_ref[0:hm, hk + c:hk + c + 512].astype(F32)
        a21 = wot_ref[hm:DM, c:c + 512].astype(F32)
        a22 = wot_ref[hm:DM, hk + c:hk + c + 512].astype(F32)
        for j, a in enumerate((a11 + a22, a21 + a22, a11 + a12, a21 - a11, a12 - a22)):
            wa_ref[j, :, c:c + 512] = a.astype(BF16)


def _out_block(i, ctx_ref, wot_ref, wa_ref, cb_ref, y_ref, o_ref):
    hm = DM // 2
    hk = H * D // 2
    q1 = BQ * i
    q2 = BQ * i + 128
    for c in range(0, hk, 512):
        b11 = ctx_ref[q1:q1 + 128, c:c + 512].astype(F32)
        b12 = ctx_ref[q2:q2 + 128, c:c + 512].astype(F32)
        b21 = ctx_ref[q1:q1 + 128, hk + c:hk + c + 512].astype(F32)
        b22 = ctx_ref[q2:q2 + 128, hk + c:hk + c + 512].astype(F32)
        for j, b in enumerate((b11 + b22, b12 - b22, b21 - b11, b11 + b12, b21 + b22)):
            cb_ref[j, :, c:c + 512] = b.astype(BF16)

    def nt(a, b):
        return jax.lax.dot_general(a, b, _NT, preferred_element_type=F32)

    m2 = nt(wa_ref[1], ctx_ref[q1:q1 + 128, 0:hk])
    m5 = nt(wa_ref[2], ctx_ref[q2:q2 + 128, hk:2 * hk])
    m3 = nt(wot_ref[0:hm, 0:hk], cb_ref[1])
    c12 = m3 + m5
    c22 = m3 - m2
    m4 = nt(wot_ref[hm:DM, hk:2 * hk], cb_ref[2])
    c21 = m2 + m4
    c11 = m4 - m5
    c22 = c22 + nt(wa_ref[3], cb_ref[3])
    m1 = nt(wa_ref[0], cb_ref[0])
    c22 = c22 + m1
    c11 = c11 + m1 + nt(wa_ref[4], cb_ref[4])
    zero = jnp.zeros((64, 128), F32)
    lane = jax.lax.broadcasted_iota(jnp.int32, (128, 128), 1)
    for r0, top, bot in ((q1, c11, c21), (q2, c12, c22)):
        bt = jnp.concatenate([zero, top, bot], axis=0).astype(BF16).T
        yv = y_ref[r0:r0 + 128, 384:512]
        o_ref[r0:r0 + 128, 0:128] = jnp.where(lane < 64, yv, bt[:, 0:128])
        o_ref[r0:r0 + 128, 128:512] = bt[:, 128:512]


def _kernel(xat_hbm, wrt_hbm, wit_hbm, xbt_hbm, c_hbm, wq_hbm, wk_hbm, wv_hbm, wot_hbm,
            fd_hbm, gf_hbm, gi_hbm, fi_hbm, out_hbm,
            xat_ref, wt_ref, fd_ref, gf_ref, gi_ref, fi_ref, y_ref, t_ref, z_ref, wn_ref,
            xbt_ref, xb_ref, c_ref, ca_ref, rawk, rawv, rawq, wkv_ref, wqh_ref,
            k_ref, v_ref, q_ref, ctx_ref, wot_ref, wa_ref, cb_ref, y_out_ref, sem, osem):
    wq32 = wq_hbm.bitcast(U32)
    wk32 = wk_hbm.bitcast(U32)
    wv32 = wv_hbm.bitcast(U32)

    def pair_copies(j, slot):
        return [
            pltpu.make_async_copy(wk32.at[:, j, :], rawk.at[slot], sem.at[16 + 3 * slot]),
            pltpu.make_async_copy(wv32.at[:, j, :], rawv.at[slot], sem.at[17 + 3 * slot]),
            pltpu.make_async_copy(wq32.at[:, j, :], rawq.at[slot], sem.at[18 + 3 * slot]),
        ]

    def copy(src, dst, s):
        return pltpu.make_async_copy(src, dst, sem.at[s])

    cp_fd = copy(fd_hbm, fd_ref, 0)
    x_cols = ((0, 512), (512, 512), (1024, 1024))
    cp_x = [copy(xat_hbm.at[:, pl.ds(o, n)], xat_ref.at[:, pl.ds(o, n)], 40 + i)
            for i, (o, n) in enumerate(x_cols)]
    cp_p0 = pair_copies(0, 0)
    cp_p1 = pair_copies(1, 1)
    cp_c = [[copy(c_hbm.at[pl.ds(o + 512 * i, 512)], c_ref.at[pl.ds(o + 512 * i, 512)], 44 + 2 * i + k)
             for k, o in enumerate((0, S // 2))] for i in range(2)]
    cp_wr = copy(wrt_hbm, wt_ref.at[0], 2)
    cp_wi = copy(wit_hbm, wt_ref.at[1], 3)
    cp_gf = copy(gf_hbm, gf_ref, 4)
    cp_gi = copy(gi_hbm, gi_ref, 5)
    cp_fi = copy(fi_hbm, fi_ref, 6)
    cp_xb = copy(xbt_hbm, xbt_ref, 7)
    for cp in ([cp_fd] + cp_x + cp_p0[:2] + cp_c[0] + [cp_wr, cp_wi, cp_gf, cp_gi]
               + cp_c[1] + [cp_fi, cp_xb, cp_p0[2]] + cp_p1):
        cp.start()

    def proj(i, w, slot):
        _kv_chunk(i, c_ref, ca_ref, wkv_ref.at[w], k_ref.at[slot], v_ref.at[slot])
        _q_chunk(i, xb_ref, wqh_ref.at[w], q_ref.at[slot])

    def relayout(i, unp, slot, w):
        _relayout_piece(i, unp, rawk.at[slot], rawv.at[slot], rawq.at[slot], wkv_ref.at[w], wqh_ref.at[w])

    def kv0(i):
        _kv_chunk(i, c_ref, ca_ref, wkv_ref.at[0], k_ref.at[0], v_ref.at[0])

    cp_fd.wait()
    for i in range(8):
        if i in (0, 2, 4):
            cp_x[i // 2].wait()
        if i == 7:
            for cp in cp_p0[:2] + cp_c[0]:
                cp.wait()
        _a_feature_dft(i, xat_ref, fd_ref, y_ref)
    for j in range(8):
        _relayout_piece(j, _lo, rawk.at[0], rawv.at[0], None, wkv_ref.at[0], None)
    _strassen_lhs(0, c_ref, ca_ref)
    for i in range(4):
        kv0(i)
        if i < 3:
            _strassen_lhs(i + 1, c_ref, ca_ref)
        _a_dft16(2 * i, -1, y_ref, t_ref)
        _a_dft16(2 * i + 1, -1, y_ref, t_ref)
        if i == 1:
            for cp in (cp_wr, cp_wi, cp_gf):
                cp.wait()
        if i >= 2:
            for a in range(8):
                _a_w_transpose(8 * (i - 2) + a, wt_ref, wn_ref)
    for q in range(16):
        if q == 8:
            for cp in [cp_gi] + cp_c[1]:
                cp.wait()
        _a_fwd_gate(q, gf_ref, t_ref, wn_ref, z_ref)
        if q >= 8 and q % 2:
            _strassen_lhs(q // 2, c_ref, ca_ref)
    for q in range(16):
        _a_inv(q, gi_ref, z_ref, y_ref)
        if q % 2:
            _relayout_piece(q // 2, _hi, rawk.at[0], rawv.at[0], None, wkv_ref.at[1], None)
    for i in range(4):
        kv0(4 + i)
        _a_dft16(2 * i, 1, y_ref, t_ref)
        _a_dft16(2 * i + 1, 1, y_ref, t_ref)
        if i == 1:
            for cp in (cp_fi, cp_xb, cp_p0[2]):
                cp.wait()
        if i >= 2:
            for j in range(2 * (i - 2), 2 * (i - 1)):
                _x_lhs(j, xbt_ref, xb_ref)
    for j in range(7):
        _relayout_q(j, _lo, rawq.at[0], wqh_ref.at[0])
        _relayout_q(j, _hi, rawq.at[0], wqh_ref.at[1])
    for i in range(8):
        _a_feature_idft(2 * i, t_ref, fi_ref, y_out_ref)
        _a_feature_idft(2 * i + 1, t_ref, fi_ref, y_out_ref)
        _q_chunk(i, xb_ref, wqh_ref.at[0], q_ref.at[0])

    cp_y = pltpu.make_async_copy(y_out_ref.at[:, pl.ds(0, 384)], out_hbm.at[:, pl.ds(0, 384)], osem.at[0])
    cp_y.start()

    cp_wo = [pltpu.make_async_copy(wot_hbm.at[h], wot_ref.at[:, pl.ds(D * h, D)], sem.at[22 + h])
             for h in range(H)]

    def head_body(h, carry):
        cur = jax.lax.rem(h, 2)
        nxt = 1 - cur
        p = h // 2 + 1
        rslot = jax.lax.rem(p, 2)

        @pl.when(jnp.logical_and(cur == 0, p < H // 2))
        def _():
            for cp in pair_copies(p, rslot):
                cp.wait()

            @pl.when(p + 1 < H // 2)
            def _():
                for cp in pair_copies(p + 1, 1 - rslot):
                    cp.start()

        @pl.when(h == 1)
        def _():
            for cp in cp_wo:
                cp.start()

        @pl.when(h == 4)
        def _():
            for cp in cp_wo:
                cp.wait()
            _out_lhs(wot_ref, wa_ref)

        sh = (16 * nxt).astype(U32)

        def unp(u):
            return pltpu.bitcast((u << sh) & jnp.uint32(0xFFFF0000), F32)

        def fill(i):
            proj(i, nxt, nxt)
            relayout(i, unp, rslot, cur)

        _attn_head(q_ref.at[cur], k_ref.at[cur], v_ref.at[cur], ctx_ref, h, fill)
        return carry

    jax.lax.fori_loop(0, H - 1, head_body, 0)

    out_cps = []

    def out_proj(i):
        r0 = BQ * i
        _out_block(i, ctx_ref, wot_ref, wa_ref, cb_ref, y_out_ref, y_out_ref)
        cp = pltpu.make_async_copy(y_out_ref.at[pl.ds(r0, BQ), :],
                                   out_hbm.at[pl.ds(r0, BQ), pl.ds(384, 512)], osem.at[1 + i])
        cp.start()
        out_cps.append(cp)

    cp_y.wait()

    def fill_last(i):
        if i > 0:
            out_proj(i - 1)

    _attn_head(q_ref.at[1], k_ref.at[1], v_ref.at[1], ctx_ref, H - 1, fill_last)
    out_proj(S // BQ - 1)
    for cp in out_cps:
        cp.wait()


def _run(A_x, A_w_r, A_w_i, B_x, B_c_kv, B_w_q, B_w_uk, B_w_uv, B_w_o):
    fd, gf, gi, fi = _dft_constants()
    any_spec = pl.BlockSpec(memory_space=pl.ANY)
    out = pl.pallas_call(
        _kernel,
        out_shape=jax.ShapeDtypeStruct((S, 2 * DM), BF16),
        in_specs=[any_spec] * 13,
        out_specs=any_spec,
        scratch_shapes=[
            pltpu.VMEM((DM, S), BF16),
            pltpu.VMEM((2, DF, S), BF16),
            pltpu.VMEM((DM, 512), BF16),
            pltpu.VMEM((16, 256, 128), BF16),
            pltpu.VMEM((16, 256, 128), BF16),
            pltpu.VMEM((512, 512), BF16),
            pltpu.VMEM((S, 512), F32),
            pltpu.VMEM((16, 128, 512), BF16),
            pltpu.VMEM((16, 128, 512), BF16),
            pltpu.VMEM((4, S, 128), BF16),
            pltpu.VMEM((DM, S), BF16),
            pltpu.VMEM((7, S // 2, DM // 2), BF16),
            pltpu.VMEM((S, DC), BF16),
            pltpu.VMEM((5, S // 2, DC // 2), BF16),
            pltpu.VMEM((2, DC, D), U32),
            pltpu.VMEM((2, DC, D), U32),
            pltpu.VMEM((2, DM, D), U32),
            pltpu.VMEM((2, 7, DC // 2, D), BF16),
            pltpu.VMEM((2, 7, DM // 2, D // 2), BF16),
            pltpu.VMEM((2, S, D), BF16),
            pltpu.VMEM((2, S, D), BF16),
            pltpu.VMEM((2, S, D), BF16),
            pltpu.VMEM((S, H * D), BF16),
            pltpu.VMEM((DM, H * D), BF16),
            pltpu.VMEM((5, DM // 2, H * D // 2), BF16),
            pltpu.VMEM((5, 128, H * D // 2), BF16),
            pltpu.VMEM((S, 512), BF16),
            pltpu.SemaphoreType.DMA((56,)),
            pltpu.SemaphoreType.DMA((16,)),
        ],
        compiler_params=pltpu.CompilerParams(vmem_limit_bytes=110 * 1024 * 1024),
    )(A_x[0].T, A_w_r.T, A_w_i.T, B_x[0].T, B_c_kv[0], B_w_q, B_w_uk, B_w_uv,
      jnp.swapaxes(B_w_o, 1, 2), fd, gf, gi, fi)
    return out[None]


@jax.jit
def pallas_concat_heads__spectral_gfnet__compressed_kv_cla__prompt_kernel(
    A_x: jax.Array,
    A_w_r: jax.Array,
    A_w_i: jax.Array,
    B_x: jax.Array,
    B_c_kv: jax.Array,
    B_w_q: jax.Array,
    B_w_uk: jax.Array,
    B_w_uv: jax.Array,
    B_w_o: jax.Array,
):
    return _run(A_x, A_w_r, A_w_i, B_x, B_c_kv, B_w_q, B_w_uk, B_w_uv, B_w_o)
```

```python
import functools

import jax
import jax.numpy as jnp
import ml_dtypes
import numpy as np
from jax.experimental import pallas as pl
from jax.experimental.pallas import tpu as pltpu

_BF = ml_dtypes.bfloat16
F32 = jnp.float32
BF16 = jnp.bfloat16
U32 = jnp.uint32

S = 2048
DM = 448
DF = 225
DC = 1024
H = 16
D = 256
BQ = 256

_NT = (((1,), (1,)), ((), ()))
_SCALE = float(np.log2(np.e) / np.sqrt(D))
_C8 = float(np.cos(np.pi / 8))
_S8 = float(np.sin(np.pi / 8))
_R2 = float(np.sqrt(0.5))


def _dft_constants():
    d = np.arange(DM)
    k2 = np.arange(DF)
    ang = 2 * np.pi * (np.outer(d, k2) % DM) / DM
    fd = np.zeros((DM, 512))
    fd[:, 0:DF] = np.cos(ang) / S
    fd[:, 256:256 + DF] = -np.sin(ang) / S
    p = np.arange(128)
    b = np.arange(128)
    gf = np.zeros((16, 256, 128))
    gi = np.zeros((16, 256, 128))
    for q in range(16):
        a = -2 * np.pi * (np.outer(16 * p + q, b) % S) / S
        gf[q, :128] = np.cos(a)
        gf[q, 128:] = np.sin(a)
        gi[q, :128] = np.cos(a).T
        gi[q, 128:] = np.sin(a).T
    cf = np.full(DF, 2.0)
    cf[0] = 1.0
    cf[-1] = 1.0
    fi = np.zeros((512, 512))
    fi[0:DF, :DM] = cf[:, None] * np.cos(ang.T) / DM
    fi[256:256 + DF, :DM] = -cf[:, None] * np.sin(ang.T) / DM
    return tuple(a.astype(np.float32).astype(_BF) for a in (fd, gf, gi, fi))


def _cmul_w(xr, xi, e, sign):
    e = e % 16
    if sign < 0:
        e = (16 - e) % 16
    q, r = divmod(e, 4)
    if r == 0:
        yr, yi = xr, xi
    elif r == 2:
        yr, yi = (xr - xi) * _R2, (xr + xi) * _R2
    elif r == 1:
        yr, yi = xr * _C8 - xi * _S8, xr * _S8 + xi * _C8
    else:
        yr, yi = xr * _S8 - xi * _C8, xr * _C8 + xi * _S8
    return yr, yi, q


def _addsub(a, b, extra=1):
    (x, sx), (y, sy) = a, b
    sy = sy * extra
    if sx > 0 and sy > 0:
        return x + y, 1
    if sx > 0 and sy < 0:
        return x - y, 1
    if sx < 0 and sy > 0:
        return y - x, 1
    return x + y, -1


def _dft4(xs, sign):
    def norm(x):
        r, i, rot = x
        rot %= 4
        if rot == 0:
            return (r, 1), (i, 1)
        if rot == 1:
            return (i, -1), (r, 1)
        if rot == 2:
            return (r, -1), (i, -1)
        return (i, 1), (r, -1)

    x = [norm(t) for t in xs]
    t0 = (_addsub(x[0][0], x[2][0]), _addsub(x[0][1], x[2][1]))
    t1 = (_addsub(x[0][0], x[2][0], -1), _addsub(x[0][1], x[2][1], -1))
    t2 = (_addsub(x[1][0], x[3][0]), _addsub(x[1][1], x[3][1]))
    t3 = (_addsub(x[1][0], x[3][0], -1), _addsub(x[1][1], x[3][1], -1))
    x0 = (_addsub(t0[0], t2[0]), _addsub(t0[1], t2[1]))
    x2 = (_addsub(t0[0], t2[0], -1), _addsub(t0[1], t2[1], -1))
    x1 = (_addsub(t1[0], t3[1], -sign), _addsub(t1[1], t3[0], sign))
    x3 = (_addsub(t1[0], t3[1], sign), _addsub(t1[1], t3[0], -sign))
    return [x0, x1, x2, x3]


def _fin(v):
    x, s = v
    return x if s > 0 else -x


def _dft16(xr, xi, sign):
    u = [[None] * 4 for _ in range(4)]
    for a0 in range(4):
        o = _dft4([(xr[a0 + 4 * a1], xi[a0 + 4 * a1], 0) for a1 in range(4)], sign)
        for q0 in range(4):
            (r, sr), (i, si) = o[q0]
            assert sr > 0 and si > 0
            u[a0][q0] = _cmul_w(r, i, a0 * q0, sign)
    yr = [None] * 16
    yi = [None] * 16
    for q0 in range(4):
        o = _dft4([u[a0][q0] for a0 in range(4)], sign)
        for q1 in range(4):
            yr[q0 + 4 * q1] = _fin(o[q1][0])
            yi[q0 + 4 * q1] = _fin(o[q1][1])
    return yr, yi


def _lo(u):
    return pltpu.bitcast(u << 16, F32)


def _hi(u):
    return pltpu.bitcast(u & jnp.uint32(0xFFFF0000), F32)


_RC = 16


def _ds(start, size):
    return pl.ds(start if isinstance(start, int) else pl.multiple_of(start, size), size)


def _loop(n, body):
    def wrapped(i, carry):
        body(i)
        return carry

    jax.lax.fori_loop(0, n, wrapped, 0)


def _a_feature_dft(i, xat_ref, fd_ref, y_ref):
    r = _ds(256 * i, 256)
    y_ref[r, :] = jnp.dot(xat_ref[:, r].T, fd_ref[...], preferred_element_type=F32)


def _a_dft16(r, sign, y_ref, t_ref):
    r = r * _RC
    for t in range(2):
        xr = [y_ref[_ds(128 * a + r, _RC), 128 * t:128 * t + 128] for a in range(16)]
        xi = [y_ref[_ds(128 * a + r, _RC), 256 + 128 * t:384 + 128 * t] for a in range(16)]
        yr, yi = _dft16(xr, xi, sign)
        for q in range(16):
            t_ref[q, _ds(r, _RC), 128 * t:128 * t + 128] = yr[q].astype(BF16)
            t_ref[q, _ds(r, _RC), 256 + 128 * t:384 + 128 * t] = yi[q].astype(BF16)


def _a_w_transpose(a, wt_ref, wn_ref):
    for ri in range(2):
        wn_ref[2 * ri, 128 * a:128 * a + 128, :] = wt_ref[ri, 0:128, 128 * a:128 * a + 128].T
        wn_ref[2 * ri + 1, 128 * a:128 * a + 128, 0:DF - 128] = (
            wt_ref[ri, 128:DF, 128 * a:128 * a + 128].T)


def _a_fwd_gate(q, gf_ref, t_ref, wn_ref, z_ref):
    lane = jax.lax.broadcasted_iota(jnp.int32, (128, 128), 1)
    wn32 = wn_ref.bitcast(U32)
    j, e = divmod(q, 2)
    unp = _lo if e == 0 else _hi
    m = jnp.dot(gf_ref[q], t_ref[q], preferred_element_type=F32)
    for t in range(2):
        xr = m[0:128, 128 * t:128 * t + 128] - m[128:256, 256 + 128 * t:384 + 128 * t]
        xi = m[128:256, 128 * t:128 * t + 128] + m[0:128, 256 + 128 * t:384 + 128 * t]
        wr = unp(wn32[t, pl.ds(j, 128, stride=8), :])
        wi = unp(wn32[2 + t, pl.ds(j, 128, stride=8), :])
        zr = xr * wr - xi * wi
        zi = xr * wi + xi * wr
        if t == 1:
            zr = jnp.where(lane < DF - 128, zr, 0.0)
            zi = jnp.where(lane < DF - 128, zi, 0.0)
        z_ref[q, :, 128 * t:128 * t + 128] = zr.astype(BF16)
        z_ref[q, :, 256 + 128 * t:384 + 128 * t] = zi.astype(BF16)


def _a_inv(q, gi_ref, z_ref, y_ref):
    m = jnp.dot(gi_ref[q], z_ref[q], preferred_element_type=F32)
    y_ref[128 * q:128 * q + 128, 0:256] = m[0:128, 0:256] + m[128:256, 256:512]
    y_ref[128 * q:128 * q + 128, 256:512] = m[0:128, 256:512] - m[128:256, 0:256]


def _a_feature_idft(a, t_ref, fi_ref, y_out_ref):
    y_out_ref[_ds(128 * a, 128), :] = jnp.dot(
        t_ref[a], fi_ref[...], preferred_element_type=F32).astype(BF16)


def _relayout_piece(i, unp, raw_k, raw_v, raw_q, wb_ref, wq_ref):
    r = 64 * i
    hc = DC // 2
    b11 = unp(raw_k[pl.ds(r, 64), :])
    b21 = unp(raw_k[pl.ds(hc + r, 64), :])
    b12 = unp(raw_v[pl.ds(r, 64), :])
    b22 = unp(raw_v[pl.ds(hc + r, 64), :])
    for j, b in enumerate(_strassen_rhs(b11, b12, b21, b22)):
        wb_ref[j, pl.ds(r, 64), :] = b.astype(BF16)
    if wq_ref is not None:
        _relayout_q(i, unp, raw_q, wq_ref)


def _strassen_rhs(b11, b12, b21, b22):
    return (b11 + b22, b11, b12 - b22, b21 - b11, b22, b11 + b12, b21 + b22)


def _relayout_q(i, unp, raw_q, wq_ref):
    hm = DM // 2
    if i < 7:
        r = 32 * i
        top = unp(raw_q[r:r + 32, :])
        bot = unp(raw_q[hm + r:hm + r + 32, :])
        for j, b in enumerate(_strassen_rhs(top[:, 0:128], top[:, 128:256], bot[:, 0:128], bot[:, 128:256])):
            wq_ref[j, r:r + 32, :] = b.astype(BF16)


def _strassen_lhs(i, c_ref, ca_ref):
    t0 = 128 * i
    b0 = S // 2 + 128 * i
    hc = DC // 2
    a11 = c_ref[_ds(t0, 128), 0:hc].astype(F32)
    a12 = c_ref[_ds(t0, 128), hc:DC].astype(F32)
    a21 = c_ref[_ds(b0, 128), 0:hc].astype(F32)
    a22 = c_ref[_ds(b0, 128), hc:DC].astype(F32)
    for j, a in enumerate((a11 + a22, a21 + a22, a11 + a12, a21 - a11, a12 - a22)):
        ca_ref[j, _ds(t0, 128), :] = a.astype(BF16)


def _strassen_products(m, emit):
    m3 = m(3)
    m5 = m(5)
    emit(12, m3 + m5)
    c22 = m3 + m(6)
    m2 = m(2)
    c22 = c22 - m2
    m4 = m(4)
    emit(21, m2 + m4)
    c11 = m4 - m5
    m1 = m(1)
    emit(22, c22 + m1)
    c11 = c11 + m1
    emit(11, c11 + m(7))


def _kv_chunk(i, c_ref, ca_ref, wb, k_ref, v_ref):
    top = _ds(128 * i, 128)
    bot = _ds(S // 2 + 128 * i, 128)
    hc = DC // 2
    lhs = [ca_ref[0, top, :], ca_ref[1, top, :], c_ref[top, 0:hc], c_ref[bot, hc:DC],
           ca_ref[2, top, :], ca_ref[3, top, :], ca_ref[4, top, :]]

    def emit(b, val):
        (k_ref if b % 10 == 1 else v_ref)[top if b < 20 else bot, :] = val.astype(BF16)

    _strassen_products(lambda j: jnp.dot(lhs[j - 1], wb[j - 1], preferred_element_type=F32), emit)


def _q_chunk(i, xa_ref, wq, q_ref):
    top = _ds(128 * i, 128)
    bot = _ds(S // 2 + 128 * i, 128)

    def emit(b, val):
        cols = pl.ds(0 if b % 10 == 1 else 128, 128)
        q_ref[top if b < 20 else bot, cols] = (val * _SCALE).astype(BF16)

    _strassen_products(
        lambda j: jnp.dot(xa_ref[j - 1, top, :], wq[j - 1], preferred_element_type=F32), emit)


def _x_lhs(i, xt_ref, xa_ref):
    hm = DM // 2
    top = _ds(256 * i, 256)
    bot = _ds(S // 2 + 256 * i, 256)
    a11 = xt_ref[0:hm, top].T.astype(F32)
    a12 = xt_ref[hm:DM, top].T.astype(F32)
    a21 = xt_ref[0:hm, bot].T.astype(F32)
    a22 = xt_ref[hm:DM, bot].T.astype(F32)
    for j, a in enumerate((a11 + a22, a21 + a22, a11, a22, a11 + a12, a21 - a11, a12 - a22)):
        xa_ref[j, top, :] = a.astype(BF16)


def _qk(i, q_ref, k_ref):
    r0 = BQ * i
    hb = BQ // 2
    row = jax.lax.broadcasted_iota(jnp.int32, (hb, hb), 0)
    col = jax.lax.broadcasted_iota(jnp.int32, (hb, hb), 1)
    tri = col <= row
    q = q_ref[r0:r0 + BQ, :]
    s_off = None
    if i > 0:
        s_off = jax.lax.dot_general(q, k_ref[0:r0, :], _NT, preferred_element_type=F32)
    s_d1 = jax.lax.dot_general(q[0:hb], k_ref[r0:r0 + hb, :], _NT, preferred_element_type=F32)
    s_d2 = jax.lax.dot_general(q[hb:BQ], k_ref[r0:r0 + BQ, :], _NT, preferred_element_type=F32)
    s_d1 = jnp.where(tri, s_d1, -1e30)
    s_d2a = s_d2[:, 0:hb]
    s_d2b = jnp.where(tri, s_d2[:, hb:BQ], -1e30)
    return s_off, s_d1, s_d2a, s_d2b


def _rowmax(x):
    return jnp.max(x, axis=1, keepdims=True)


def _rowsum(x):
    return jnp.sum(x, axis=1, keepdims=True)


def _pv(i, s, v_ref, ctx_ref, cols):
    r0 = BQ * i
    hb = BQ // 2
    s_off, s_d1, s_d2a, s_d2b = s
    m1 = _rowmax(s_d1)
    m2 = _rowmax(jnp.maximum(s_d2a, s_d2b))
    if s_off is not None:
        mo = _rowmax(s_off)
        m1 = jnp.maximum(m1, mo[0:hb])
        m2 = jnp.maximum(m2, mo[hb:BQ])
    p1 = jnp.exp2(s_d1 - m1)
    p2a = jnp.exp2(s_d2a - m2)
    p2b = jnp.exp2(s_d2b - m2)
    l1 = _rowsum(p1)
    l2 = _rowsum(p2a + p2b)
    o1 = jnp.dot(p1.astype(BF16), v_ref[r0:r0 + hb, :], preferred_element_type=F32)
    p2 = jnp.concatenate([p2a.astype(BF16), p2b.astype(BF16)], axis=1)
    o2 = jnp.dot(p2, v_ref[r0:r0 + BQ, :], preferred_element_type=F32)
    if s_off is not None:
        m = jnp.concatenate([m1, m2], axis=0)
        po = jnp.exp2(s_off - m)
        lo = _rowsum(po)
        oo = jnp.dot(po.astype(BF16), v_ref[0:r0, :], preferred_element_type=F32)
        l1 = l1 + lo[0:hb]
        l2 = l2 + lo[hb:BQ]
        o1 = o1 + oo[0:hb]
        o2 = o2 + oo[hb:BQ]
    ctx_ref[r0:r0 + hb, cols] = (o1 * (1.0 / l1)).astype(BF16)
    ctx_ref[r0 + hb:r0 + BQ, cols] = (o2 * (1.0 / l2)).astype(BF16)


def _attn_head(q_ref, k_ref, v_ref, ctx_ref, h, filler):
    cols = pl.ds(h * D if isinstance(h, int) else pl.multiple_of(h * D, D), D)
    for i in range(S // BQ):
        s = _qk(i, q_ref, k_ref)
        filler(i)
        _pv(i, s, v_ref, ctx_ref, cols)


def _out_lhs(wot_ref, wa_ref):
    hm = DM // 2
    hk = H * D // 2
    for c in range(0, hk, 512):
        a11 = wot_ref[0:hm, c:c + 512].astype(F32)
        a12 = wot_ref[0:hm, hk + c:hk + c + 512].astype(F32)
        a21 = wot_ref[hm:DM, c:c + 512].astype(F32)
        a22 = wot_ref[hm:DM, hk + c:hk + c + 512].astype(F32)
        for j, a in enumerate((a11 + a22, a21 + a22, a11 + a12, a21 - a11, a12 - a22)):
            wa_ref[j, :, c:c + 512] = a.astype(BF16)


def _out_block(i, ctx_ref, wot_ref, wa_ref, cb_ref, y_ref, o_ref):
    hm = DM // 2
    hk = H * D // 2
    q1 = _ds(BQ * i, 128)
    q2 = _ds(BQ * i + 128, 128)
    for c in range(0, hk, 256):
        b11 = ctx_ref[q1, c:c + 256].astype(F32)
        b12 = ctx_ref[q2, c:c + 256].astype(F32)
        b21 = ctx_ref[q1, hk + c:hk + c + 256].astype(F32)
        b22 = ctx_ref[q2, hk + c:hk + c + 256].astype(F32)
        for j, b in enumerate((b11 + b22, b12 - b22, b21 - b11, b11 + b12, b21 + b22)):
            cb_ref[j, :, c:c + 256] = b.astype(BF16)

    def nt(a, b):
        return jax.lax.dot_general(a, b, _NT, preferred_element_type=F32)

    m2 = nt(wa_ref[1], ctx_ref[q1, 0:hk])
    m5 = nt(wa_ref[2], ctx_ref[q2, hk:2 * hk])
    m3 = nt(wot_ref[0:hm, 0:hk], cb_ref[1])
    c12 = m3 + m5
    c22 = m3 - m2
    m4 = nt(wot_ref[hm:DM, hk:2 * hk], cb_ref[2])
    c21 = m2 + m4
    c11 = m4 - m5
    c22 = c22 + nt(wa_ref[3], cb_ref[3])
    m1 = nt(wa_ref[0], cb_ref[0])
    c22 = c22 + m1
    c11 = c11 + m1 + nt(wa_ref[4], cb_ref[4])
    zero = jnp.zeros((64, 128), F32)
    lane = jax.lax.broadcasted_iota(jnp.int32, (128, 128), 1)
    for r0, top, bot in ((q1, c11, c21), (q2, c12, c22)):
        bt = jnp.concatenate([zero, top, bot], axis=0).astype(BF16).T
        yv = y_ref[r0, 384:512]
        o_ref[r0, 0:128] = jnp.where(lane < 64, yv, bt[:, 0:128])
        o_ref[r0, 128:512] = bt[:, 128:512]


def _kernel(xat_hbm, wrt_hbm, wit_hbm, xbt_hbm, c_hbm, wq_hbm, wk_hbm, wv_hbm, wot_hbm,
            fd_hbm, gf_hbm, gi_hbm, fi_hbm, out_hbm,
            xat_ref, wt_ref, fd_ref, gf_ref, gi_ref, fi_ref, y_ref, t_ref, z_ref, wn_ref,
            xbt_ref, xb_ref, c_ref, ca_ref, rawk, rawv, rawq, wkv_ref, wqh_ref,
            k_ref, v_ref, q_ref, ctx_ref, wot_ref, wa_ref, cb_ref, y_out_ref, sem, osem):
    wq32 = wq_hbm.bitcast(U32)
    wk32 = wk_hbm.bitcast(U32)
    wv32 = wv_hbm.bitcast(U32)

    def pair_copies(j, slot):
        return [
            pltpu.make_async_copy(wk32.at[:, j, :], rawk.at[slot], sem.at[16 + 3 * slot]),
            pltpu.make_async_copy(wv32.at[:, j, :], rawv.at[slot], sem.at[17 + 3 * slot]),
            pltpu.make_async_copy(wq32.at[:, j, :], rawq.at[slot], sem.at[18 + 3 * slot]),
        ]

    def copy(src, dst, s):
        return pltpu.make_async_copy(src, dst, sem.at[s])

    cp_fd = copy(fd_hbm, fd_ref, 0)
    x_cols = ((0, 512), (512, 512), (1024, 1024))
    cp_x = [copy(xat_hbm.at[:, pl.ds(o, n)], xat_ref.at[:, pl.ds(o, n)], 40 + i)
            for i, (o, n) in enumerate(x_cols)]
    cp_p0 = pair_copies(0, 0)
    cp_p1 = pair_copies(1, 1)
    cp_c = [[copy(c_hbm.at[pl.ds(o + 512 * i, 512)], c_ref.at[pl.ds(o + 512 * i, 512)], 44 + 2 * i + k)
             for k, o in enumerate((0, S // 2))] for i in range(2)]
    cp_wr = copy(wrt_hbm, wt_ref.at[0], 2)
    cp_wi = copy(wit_hbm, wt_ref.at[1], 3)
    cp_gf = copy(gf_hbm, gf_ref, 4)
    cp_gi = copy(gi_hbm, gi_ref, 5)
    cp_fi = copy(fi_hbm, fi_ref, 6)
    cp_xb = copy(xbt_hbm, xbt_ref, 7)
    for cp in ([cp_fd] + cp_x + cp_p0[:2] + cp_c[0] + [cp_wr, cp_wi, cp_gf, cp_gi]
               + cp_c[1] + [cp_fi, cp_xb, cp_p0[2]] + cp_p1):
        cp.start()

    def proj(i, w, slot):
        _kv_chunk(i, c_ref, ca_ref, wkv_ref.at[w], k_ref.at[slot], v_ref.at[slot])
        _q_chunk(i, xb_ref, wqh_ref.at[w], q_ref.at[slot])

    def relayout(i, unp, slot, w):
        _relayout_piece(i, unp, rawk.at[slot], rawv.at[slot], rawq.at[slot], wkv_ref.at[w], wqh_ref.at[w])

    def kv0(i):
        _kv_chunk(i, c_ref, ca_ref, wkv_ref.at[0], k_ref.at[0], v_ref.at[0])

    cp_fd.wait()
    cp_x[0].wait()

    def a1(ii):
        @pl.when(ii == 1)
        def _():
            cp_x[1].wait()

        @pl.when(ii == 2)
        def _():
            cp_x[2].wait()

        _a_feature_dft(2 * ii, xat_ref, fd_ref, y_ref)
        _a_feature_dft(2 * ii + 1, xat_ref, fd_ref, y_ref)

    _loop(4, a1)
    for cp in cp_p0[:2] + cp_c[0]:
        cp.wait()
    for j in range(8):
        _relayout_piece(j, _lo, rawk.at[0], rawv.at[0], None, wkv_ref.at[0], None)

    def kv_dft(base, sign):
        def body(i):
            _strassen_lhs(base + i, c_ref, ca_ref)
            kv0(base + i)
            _a_dft16(2 * i, sign, y_ref, t_ref)
            _a_dft16(2 * i + 1, sign, y_ref, t_ref)
        return body

    _loop(4, kv_dft(0, -1))
    for cp in (cp_wr, cp_wi, cp_gf):
        cp.wait()
    for a in range(16):
        _a_w_transpose(a, wt_ref, wn_ref)
    for q in range(16):
        _a_fwd_gate(q, gf_ref, t_ref, wn_ref, z_ref)
    for cp in [cp_gi] + cp_c[1]:
        cp.wait()
    for q in range(16):
        _a_inv(q, gi_ref, z_ref, y_ref)
        if q % 2:
            _relayout_piece(q // 2, _hi, rawk.at[0], rawv.at[0], None, wkv_ref.at[1], None)
    _loop(4, kv_dft(4, 1))
    for cp in (cp_fi, cp_xb, cp_p0[2]):
        cp.wait()

    def a5(i):
        for a in range(4):
            _a_feature_idft(4 * i + a, t_ref, fi_ref, y_out_ref)
        _x_lhs(i, xbt_ref, xb_ref)

    _loop(4, a5)
    for j in range(7):
        _relayout_q(j, _lo, rawq.at[0], wqh_ref.at[0])
        _relayout_q(j, _hi, rawq.at[0], wqh_ref.at[1])
    for i in range(8):
        _q_chunk(i, xb_ref, wqh_ref.at[0], q_ref.at[0])

    cp_y = pltpu.make_async_copy(y_out_ref.at[:, pl.ds(0, 384)], out_hbm.at[:, pl.ds(0, 384)], osem.at[0])
    cp_y.start()

    cp_wo = [pltpu.make_async_copy(wot_hbm.at[h], wot_ref.at[:, pl.ds(D * h, D)], sem.at[22 + h])
             for h in range(H)]

    def head_body(h, carry):
        cur = jax.lax.rem(h, 2)
        nxt = 1 - cur
        p = h // 2 + 1
        rslot = jax.lax.rem(p, 2)

        @pl.when(jnp.logical_and(cur == 0, p < H // 2))
        def _():
            for cp in pair_copies(p, rslot):
                cp.wait()

            @pl.when(p + 1 < H // 2)
            def _():
                for cp in pair_copies(p + 1, 1 - rslot):
                    cp.start()

        @pl.when(h == 1)
        def _():
            for cp in cp_wo:
                cp.start()

        @pl.when(h == 4)
        def _():
            for cp in cp_wo:
                cp.wait()
            _out_lhs(wot_ref, wa_ref)

        sh = (16 * nxt).astype(U32)

        def unp(u):
            return pltpu.bitcast((u << sh) & jnp.uint32(0xFFFF0000), F32)

        def fill(i):
            proj(i, nxt, nxt)
            relayout(i, unp, rslot, cur)

        _attn_head(q_ref.at[cur], k_ref.at[cur], v_ref.at[cur], ctx_ref, h, fill)
        return carry

    jax.lax.fori_loop(0, H - 1, head_body, 0)

    def out_copy(i):
        rows = _ds(BQ * i, BQ)
        return pltpu.make_async_copy(y_out_ref.at[rows, :], out_hbm.at[rows, pl.ds(384, 512)], osem.at[1 + i])

    def out_proj(i):
        _out_block(i, ctx_ref, wot_ref, wa_ref, cb_ref, y_out_ref, y_out_ref)
        out_copy(i).start()

    cp_y.wait()

    def fill_last(i):
        if 0 < i < 7:
            out_proj(i - 1)

    _attn_head(q_ref.at[1], k_ref.at[1], v_ref.at[1], ctx_ref, H - 1, fill_last)
    _loop(2, lambda i: out_proj(6 + i))
    for i in range(S // BQ):
        out_copy(i).wait()


def _run(A_x, A_w_r, A_w_i, B_x, B_c_kv, B_w_q, B_w_uk, B_w_uv, B_w_o):
    fd, gf, gi, fi = _dft_constants()
    any_spec = pl.BlockSpec(memory_space=pl.ANY)
    out = pl.pallas_call(
        _kernel,
        out_shape=jax.ShapeDtypeStruct((S, 2 * DM), BF16),
        in_specs=[any_spec] * 13,
        out_specs=any_spec,
        scratch_shapes=[
            pltpu.VMEM((DM, S), BF16),
            pltpu.VMEM((2, DF, S), BF16),
            pltpu.VMEM((DM, 512), BF16),
            pltpu.VMEM((16, 256, 128), BF16),
            pltpu.VMEM((16, 256, 128), BF16),
            pltpu.VMEM((512, 512), BF16),
            pltpu.VMEM((S, 512), F32),
            pltpu.VMEM((16, 128, 512), BF16),
            pltpu.VMEM((16, 128, 512), BF16),
            pltpu.VMEM((4, S, 128), BF16),
            pltpu.VMEM((DM, S), BF16),
            pltpu.VMEM((7, S // 2, DM // 2), BF16),
            pltpu.VMEM((S, DC), BF16),
            pltpu.VMEM((5, S // 2, DC // 2), BF16),
            pltpu.VMEM((2, DC, D), U32),
            pltpu.VMEM((2, DC, D), U32),
            pltpu.VMEM((2, DM, D), U32),
            pltpu.VMEM((2, 7, DC // 2, D), BF16),
            pltpu.VMEM((2, 7, DM // 2, D // 2), BF16),
            pltpu.VMEM((2, S, D), BF16),
            pltpu.VMEM((2, S, D), BF16),
            pltpu.VMEM((2, S, D), BF16),
            pltpu.VMEM((S, H * D), BF16),
            pltpu.VMEM((DM, H * D), BF16),
            pltpu.VMEM((5, DM // 2, H * D // 2), BF16),
            pltpu.VMEM((5, 128, H * D // 2), BF16),
            pltpu.VMEM((S, 512), BF16),
            pltpu.SemaphoreType.DMA((56,)),
            pltpu.SemaphoreType.DMA((16,)),
        ],
        compiler_params=pltpu.CompilerParams(vmem_limit_bytes=110 * 1024 * 1024),
    )(A_x[0].T, A_w_r.T, A_w_i.T, B_x[0].T, B_c_kv[0], B_w_q, B_w_uk, B_w_uv,
      jnp.swapaxes(B_w_o, 1, 2), fd, gf, gi, fi)
    return out[None]


@jax.jit
def pallas_concat_heads__spectral_gfnet__compressed_kv_cla__prompt_kernel(
    A_x: jax.Array,
    A_w_r: jax.Array,
    A_w_i: jax.Array,
    B_x: jax.Array,
    B_c_kv: jax.Array,
    B_w_q: jax.Array,
    B_w_uk: jax.Array,
    B_w_uv: jax.Array,
    B_w_o: jax.Array,
):
    return _run(A_x, A_w_r, A_w_i, B_x, B_c_kv, B_w_q, B_w_uk, B_w_uv, B_w_o)
```

```python
import jax
import jax.numpy as jnp
import ml_dtypes
import numpy as np
from jax.experimental import pallas as pl
from jax.experimental.pallas import tpu as pltpu

_BF = ml_dtypes.bfloat16
F32 = jnp.float32
BF16 = jnp.bfloat16
U32 = jnp.uint32

S = 2048
DM = 448
DF = 225
DC = 1024
H = 16
D = 256
BQ = 256

_NT = (((1,), (1,)), ((), ()))
_SCALE = float(np.log2(np.e) / np.sqrt(D))
_C8 = float(np.cos(np.pi / 8))
_S8 = float(np.sin(np.pi / 8))
_R2 = float(np.sqrt(0.5))


def _dft_constants():
    d = np.arange(DM)
    k2 = np.arange(DF)
    ang = 2 * np.pi * (np.outer(d, k2) % DM) / DM
    fd = np.zeros((DM, 512))
    fd[:, 0:DF] = np.cos(ang) / S
    fd[:, 256:256 + DF] = -np.sin(ang) / S
    p = np.arange(128)
    b = np.arange(128)
    gf = np.zeros((16, 256, 128))
    gi = np.zeros((16, 256, 128))
    for q in range(16):
        a = -2 * np.pi * (np.outer(16 * p + q, b) % S) / S
        gf[q, :128] = np.cos(a)
        gf[q, 128:] = np.sin(a)
        gi[q, :128] = np.cos(a).T
        gi[q, 128:] = np.sin(a).T
    cf = np.full(DF, 2.0)
    cf[0] = 1.0
    cf[-1] = 1.0
    fi = np.zeros((512, 512))
    fi[0:DF, :DM] = cf[:, None] * np.cos(ang.T) / DM
    fi[256:256 + DF, :DM] = -cf[:, None] * np.sin(ang.T) / DM
    return tuple(a.astype(np.float32).astype(_BF) for a in (fd, gf, gi, fi))


def _cmul_w(xr, xi, e, sign):
    e = e % 16
    if sign < 0:
        e = (16 - e) % 16
    q, r = divmod(e, 4)
    if r == 0:
        yr, yi = xr, xi
    elif r == 2:
        yr, yi = (xr - xi) * _R2, (xr + xi) * _R2
    elif r == 1:
        yr, yi = xr * _C8 - xi * _S8, xr * _S8 + xi * _C8
    else:
        yr, yi = xr * _S8 - xi * _C8, xr * _C8 + xi * _S8
    return yr, yi, q


def _addsub(a, b, extra=1):
    (x, sx), (y, sy) = a, b
    sy = sy * extra
    if sx > 0 and sy > 0:
        return x + y, 1
    if sx > 0 and sy < 0:
        return x - y, 1
    if sx < 0 and sy > 0:
        return y - x, 1
    return x + y, -1


def _dft4(xs, sign):
    def norm(x):
        r, i, rot = x
        rot %= 4
        if rot == 0:
            return (r, 1), (i, 1)
        if rot == 1:
            return (i, -1), (r, 1)
        if rot == 2:
            return (r, -1), (i, -1)
        return (i, 1), (r, -1)

    x = [norm(t) for t in xs]
    t0 = (_addsub(x[0][0], x[2][0]), _addsub(x[0][1], x[2][1]))
    t1 = (_addsub(x[0][0], x[2][0], -1), _addsub(x[0][1], x[2][1], -1))
    t2 = (_addsub(x[1][0], x[3][0]), _addsub(x[1][1], x[3][1]))
    t3 = (_addsub(x[1][0], x[3][0], -1), _addsub(x[1][1], x[3][1], -1))
    x0 = (_addsub(t0[0], t2[0]), _addsub(t0[1], t2[1]))
    x2 = (_addsub(t0[0], t2[0], -1), _addsub(t0[1], t2[1], -1))
    x1 = (_addsub(t1[0], t3[1], -sign), _addsub(t1[1], t3[0], sign))
    x3 = (_addsub(t1[0], t3[1], sign), _addsub(t1[1], t3[0], -sign))
    return [x0, x1, x2, x3]


def _fin(v):
    x, s = v
    return x if s > 0 else -x


def _dft16(xr, xi, sign):
    u = [[None] * 4 for _ in range(4)]
    for a0 in range(4):
        o = _dft4([(xr[a0 + 4 * a1], xi[a0 + 4 * a1], 0) for a1 in range(4)], sign)
        for q0 in range(4):
            (r, sr), (i, si) = o[q0]
            assert sr > 0 and si > 0
            u[a0][q0] = _cmul_w(r, i, a0 * q0, sign)
    yr = [None] * 16
    yi = [None] * 16
    for q0 in range(4):
        o = _dft4([u[a0][q0] for a0 in range(4)], sign)
        for q1 in range(4):
            yr[q0 + 4 * q1] = _fin(o[q1][0])
            yi[q0 + 4 * q1] = _fin(o[q1][1])
    return yr, yi


def _lo(u):
    return pltpu.bitcast(u << 16, F32)


def _hi(u):
    return pltpu.bitcast(u & jnp.uint32(0xFFFF0000), F32)


_RC = 16


def _ds(start, size):
    return pl.ds(start if isinstance(start, int) else pl.multiple_of(start, size), size)


def _loop(n, body):
    def wrapped(i, carry):
        body(i)
        return carry

    jax.lax.fori_loop(0, n, wrapped, 0)


def _a_feature_dft(i, xat_ref, fd_ref, y_ref):
    r = _ds(256 * i, 256)
    y_ref[r, :] = jnp.dot(xat_ref[:, r].T, fd_ref[...], preferred_element_type=F32)


def _a_dft16(r, sign, y_ref, t_ref):
    r = r * _RC
    for t in range(2):
        xr = [y_ref[_ds(128 * a + r, _RC), 128 * t:128 * t + 128] for a in range(16)]
        xi = [y_ref[_ds(128 * a + r, _RC), 256 + 128 * t:384 + 128 * t] for a in range(16)]
        yr, yi = _dft16(xr, xi, sign)
        for q in range(16):
            t_ref[q, _ds(r, _RC), 128 * t:128 * t + 128] = yr[q].astype(BF16)
            t_ref[q, _ds(r, _RC), 256 + 128 * t:384 + 128 * t] = yi[q].astype(BF16)


def _a_w_transpose(a, wt_ref, wn_ref):
    for ri in range(2):
        wn_ref[2 * ri, 128 * a:128 * a + 128, :] = wt_ref[ri, 0:128, 128 * a:128 * a + 128].T
        wn_ref[2 * ri + 1, 128 * a:128 * a + 128, 0:DF - 128] = (
            wt_ref[ri, 128:DF, 128 * a:128 * a + 128].T)


def _a_fwd_gate(q, gf_ref, t_ref, wn_ref, z_ref):
    lane = jax.lax.broadcasted_iota(jnp.int32, (128, 128), 1)
    wn32 = wn_ref.bitcast(U32)
    j, e = divmod(q, 2)
    unp = _lo if e == 0 else _hi
    m = jnp.dot(gf_ref[q], t_ref[q], preferred_element_type=F32)
    for t in range(2):
        xr = m[0:128, 128 * t:128 * t + 128] - m[128:256, 256 + 128 * t:384 + 128 * t]
        xi = m[128:256, 128 * t:128 * t + 128] + m[0:128, 256 + 128 * t:384 + 128 * t]
        wr = unp(wn32[t, pl.ds(j, 128, stride=8), :])
        wi = unp(wn32[2 + t, pl.ds(j, 128, stride=8), :])
        zr = xr * wr - xi * wi
        zi = xr * wi + xi * wr
        if t == 1:
            zr = jnp.where(lane < DF - 128, zr, 0.0)
            zi = jnp.where(lane < DF - 128, zi, 0.0)
        z_ref[q, :, 128 * t:128 * t + 128] = zr.astype(BF16)
        z_ref[q, :, 256 + 128 * t:384 + 128 * t] = zi.astype(BF16)


def _a_inv(q, gi_ref, z_ref, y_ref):
    m = jnp.dot(gi_ref[q], z_ref[q], preferred_element_type=F32)
    y_ref[128 * q:128 * q + 128, 0:256] = m[0:128, 0:256] + m[128:256, 256:512]
    y_ref[128 * q:128 * q + 128, 256:512] = m[0:128, 256:512] - m[128:256, 0:256]


def _a_feature_idft(a, t_ref, fi_ref, y_out_ref):
    y_out_ref[_ds(128 * a, 128), :] = jnp.dot(
        t_ref[a], fi_ref[...], preferred_element_type=F32).astype(BF16)


def _relayout_piece(i, unp, raw_k, raw_v, raw_q, wb_ref, wq_ref):
    r = 64 * i
    hc = DC // 2
    b11 = unp(raw_k[pl.ds(r, 64), :])
    b21 = unp(raw_k[pl.ds(hc + r, 64), :])
    b12 = unp(raw_v[pl.ds(r, 64), :])
    b22 = unp(raw_v[pl.ds(hc + r, 64), :])
    for j, b in enumerate(_strassen_rhs(b11, b12, b21, b22)):
        wb_ref[j, pl.ds(r, 64), :] = b.astype(BF16)
    if wq_ref is not None:
        _relayout_q(i, unp, raw_q, wq_ref)


def _strassen_rhs(b11, b12, b21, b22):
    return (b11 + b22, b11, b12 - b22, b21 - b11, b22, b11 + b12, b21 + b22)


def _relayout_q(i, unp, raw_q, wq_ref):
    hm = DM // 2
    if i < 7:
        r = 32 * i
        top = unp(raw_q[r:r + 32, :])
        bot = unp(raw_q[hm + r:hm + r + 32, :])
        for j, b in enumerate(_strassen_rhs(top[:, 0:128], top[:, 128:256], bot[:, 0:128], bot[:, 128:256])):
            wq_ref[j, r:r + 32, :] = b.astype(BF16)


def _strassen_lhs(i, c_ref, ca_ref):
    t0 = 128 * i
    b0 = S // 2 + 128 * i
    hc = DC // 2
    a11 = c_ref[_ds(t0, 128), 0:hc].astype(F32)
    a12 = c_ref[_ds(t0, 128), hc:DC].astype(F32)
    a21 = c_ref[_ds(b0, 128), 0:hc].astype(F32)
    a22 = c_ref[_ds(b0, 128), hc:DC].astype(F32)
    for j, a in enumerate((a11 + a22, a21 + a22, a11 + a12, a21 - a11, a12 - a22)):
        ca_ref[j, _ds(t0, 128), :] = a.astype(BF16)


def _strassen_products(m, emit):
    m3 = m(3)
    m5 = m(5)
    emit(12, m3 + m5)
    c22 = m3 + m(6)
    m2 = m(2)
    c22 = c22 - m2
    m4 = m(4)
    emit(21, m2 + m4)
    c11 = m4 - m5
    m1 = m(1)
    emit(22, c22 + m1)
    c11 = c11 + m1
    emit(11, c11 + m(7))


def _kv_chunk(i, c_ref, ca_ref, wb, k_ref, v_ref):
    top = _ds(128 * i, 128)
    bot = _ds(S // 2 + 128 * i, 128)
    hc = DC // 2
    lhs = [ca_ref[0, top, :], ca_ref[1, top, :], c_ref[top, 0:hc], c_ref[bot, hc:DC],
           ca_ref[2, top, :], ca_ref[3, top, :], ca_ref[4, top, :]]

    def emit(b, val):
        (k_ref if b % 10 == 1 else v_ref)[top if b < 20 else bot, :] = val.astype(BF16)

    _strassen_products(lambda j: jnp.dot(lhs[j - 1], wb[j - 1], preferred_element_type=F32), emit)


def _q_chunk(i, xa_ref, wq, q_ref):
    top = _ds(128 * i, 128)
    bot = _ds(S // 2 + 128 * i, 128)

    def emit(b, val):
        cols = pl.ds(0 if b % 10 == 1 else 128, 128)
        q_ref[top if b < 20 else bot, cols] = (val * _SCALE).astype(BF16)

    _strassen_products(
        lambda j: jnp.dot(xa_ref[j - 1, top, :], wq[j - 1], preferred_element_type=F32), emit)


def _x_lhs(i, xt_ref, xa_ref):
    hm = DM // 2
    top = _ds(256 * i, 256)
    bot = _ds(S // 2 + 256 * i, 256)
    a11 = xt_ref[0:hm, top].T.astype(F32)
    a12 = xt_ref[hm:DM, top].T.astype(F32)
    a21 = xt_ref[0:hm, bot].T.astype(F32)
    a22 = xt_ref[hm:DM, bot].T.astype(F32)
    for j, a in enumerate((a11 + a22, a21 + a22, a11, a22, a11 + a12, a21 - a11, a12 - a22)):
        xa_ref[j, top, :] = a.astype(BF16)


def _qk(i, q_ref, k_ref):
    r0 = BQ * i
    hb = BQ // 2
    row = jax.lax.broadcasted_iota(jnp.int32, (hb, hb), 0)
    col = jax.lax.broadcasted_iota(jnp.int32, (hb, hb), 1)
    tri = col <= row
    q = q_ref[r0:r0 + BQ, :]
    s_off = None
    if i > 0:
        s_off = jax.lax.dot_general(q, k_ref[0:r0, :], _NT, preferred_element_type=F32)
    s_d1 = jax.lax.dot_general(q[0:hb], k_ref[r0:r0 + hb, :], _NT, preferred_element_type=F32)
    s_d2 = jax.lax.dot_general(q[hb:BQ], k_ref[r0:r0 + BQ, :], _NT, preferred_element_type=F32)
    s_d1 = jnp.where(tri, s_d1, -1e30)
    s_d2a = s_d2[:, 0:hb]
    s_d2b = jnp.where(tri, s_d2[:, hb:BQ], -1e30)
    return s_off, s_d1, s_d2a, s_d2b


def _rowmax(x):
    return jnp.max(x, axis=1, keepdims=True)


def _rowsum(x):
    return jnp.sum(x, axis=1, keepdims=True)


def _softmax(s):
    hb = BQ // 2
    s_off, s_d1, s_d2a, s_d2b = s
    m1 = _rowmax(s_d1)
    m2 = _rowmax(jnp.maximum(s_d2a, s_d2b))
    if s_off is not None:
        mo = _rowmax(s_off)
        m1 = jnp.maximum(m1, mo[0:hb])
        m2 = jnp.maximum(m2, mo[hb:BQ])
    p1 = jnp.exp2(s_d1 - m1)
    p2a = jnp.exp2(s_d2a - m2)
    p2b = jnp.exp2(s_d2b - m2)
    l1 = _rowsum(p1)
    l2 = _rowsum(p2a + p2b)
    p2 = jnp.concatenate([p2a.astype(BF16), p2b.astype(BF16)], axis=1)
    po = None
    if s_off is not None:
        m = jnp.concatenate([m1, m2], axis=0)
        po = jnp.exp2(s_off - m)
        lo = _rowsum(po)
        po = po.astype(BF16)
        l1 = l1 + lo[0:hb]
        l2 = l2 + lo[hb:BQ]
    return po, p1.astype(BF16), p2, 1.0 / l1, 1.0 / l2


def _pv(i, p, v_ref, ctx_ref, cols):
    r0 = BQ * i
    hb = BQ // 2
    po, p1, p2, r1, r2 = p
    o1 = jnp.dot(p1, v_ref[r0:r0 + hb, :], preferred_element_type=F32)
    o2 = jnp.dot(p2, v_ref[r0:r0 + BQ, :], preferred_element_type=F32)
    if po is not None:
        oo = jnp.dot(po, v_ref[0:r0, :], preferred_element_type=F32)
        o1 = o1 + oo[0:hb]
        o2 = o2 + oo[hb:BQ]
    ctx_ref[r0:r0 + hb, cols] = (o1 * r1).astype(BF16)
    ctx_ref[r0 + hb:r0 + BQ, cols] = (o2 * r2).astype(BF16)


def _attn_head(q_ref, k_ref, v_ref, ctx_ref, h, filler, plan=None):
    cols = pl.ds(h * D if isinstance(h, int) else pl.multiple_of(h * D, D), D)
    plan = 'q7 q6 f0 p7 q5 f1 p6 q4 f2 p5 q3 f3 p4 q2 f4 p3 q1 f5 p2 q0 f6 p1 f7 p0' if plan is None else plan
    st = {}
    for op in plan.split():
        i = int(op[1])
        if op[0] == 'q':
            st[i] = _softmax(_qk(i, q_ref, k_ref))
        elif op[0] == 'f':
            filler(i)
        else:
            _pv(i, st.pop(i), v_ref, ctx_ref, cols)


def _out_lhs(wot_ref, wa_ref):
    hm = DM // 2
    hk = H * D // 2
    for c in range(0, hk, 512):
        a11 = wot_ref[0:hm, c:c + 512].astype(F32)
        a12 = wot_ref[0:hm, hk + c:hk + c + 512].astype(F32)
        a21 = wot_ref[hm:DM, c:c + 512].astype(F32)
        a22 = wot_ref[hm:DM, hk + c:hk + c + 512].astype(F32)
        for j, a in enumerate((a11 + a22, a21 + a22, a11 + a12, a21 - a11, a12 - a22)):
            wa_ref[j, :, c:c + 512] = a.astype(BF16)


def _out_block(i, ctx_ref, wot_ref, wa_ref, cb_ref, y_ref, o_ref):
    hm = DM // 2
    hk = H * D // 2
    q1 = _ds(BQ * i, 128)
    q2 = _ds(BQ * i + 128, 128)
    for c in range(0, hk, 256):
        b11 = ctx_ref[q1, c:c + 256].astype(F32)
        b12 = ctx_ref[q2, c:c + 256].astype(F32)
        b21 = ctx_ref[q1, hk + c:hk + c + 256].astype(F32)
        b22 = ctx_ref[q2, hk + c:hk + c + 256].astype(F32)
        for j, b in enumerate((b11 + b22, b12 - b22, b21 - b11, b11 + b12, b21 + b22)):
            cb_ref[j, :, c:c + 256] = b.astype(BF16)

    def nt(a, b):
        return jax.lax.dot_general(a, b, _NT, preferred_element_type=F32)

    m2 = nt(wa_ref[1], ctx_ref[q1, 0:hk])
    m5 = nt(wa_ref[2], ctx_ref[q2, hk:2 * hk])
    m3 = nt(wot_ref[0:hm, 0:hk], cb_ref[1])
    c12 = m3 + m5
    c22 = m3 - m2
    m4 = nt(wot_ref[hm:DM, hk:2 * hk], cb_ref[2])
    c21 = m2 + m4
    c11 = m4 - m5
    c22 = c22 + nt(wa_ref[3], cb_ref[3])
    m1 = nt(wa_ref[0], cb_ref[0])
    c22 = c22 + m1
    c11 = c11 + m1 + nt(wa_ref[4], cb_ref[4])
    zero = jnp.zeros((64, 128), F32)
    lane = jax.lax.broadcasted_iota(jnp.int32, (128, 128), 1)
    for r0, top, bot in ((q1, c11, c21), (q2, c12, c22)):
        bt = jnp.concatenate([zero, top, bot], axis=0).astype(BF16).T
        yv = y_ref[r0, 384:512]
        o_ref[r0, 0:128] = jnp.where(lane < 64, yv, bt[:, 0:128])
        o_ref[r0, 128:512] = bt[:, 128:512]


def _kernel(xat_hbm, wrt_hbm, wit_hbm, xbt_hbm, c_hbm, wq_hbm, wk_hbm, wv_hbm, wot_hbm,
            fd_hbm, gf_hbm, gi_hbm, fi_hbm, out_hbm,
            xat_ref, wt_ref, fd_ref, gf_ref, gi_ref, fi_ref, y_ref, t_ref, z_ref, wn_ref,
            xbt_ref, xb_ref, c_ref, ca_ref, rawk, rawv, rawq, wkv_ref, wqh_ref,
            k_ref, v_ref, q_ref, ctx_ref, wot_ref, wa_ref, cb_ref, y_out_ref, sem, osem):
    wq32 = wq_hbm.bitcast(U32)
    wk32 = wk_hbm.bitcast(U32)
    wv32 = wv_hbm.bitcast(U32)

    def pair_copies(j, slot):
        return [
            pltpu.make_async_copy(wk32.at[:, j, :], rawk.at[slot], sem.at[16 + 3 * slot]),
            pltpu.make_async_copy(wv32.at[:, j, :], rawv.at[slot], sem.at[17 + 3 * slot]),
            pltpu.make_async_copy(wq32.at[:, j, :], rawq.at[slot], sem.at[18 + 3 * slot]),
        ]

    def copy(src, dst, s):
        return pltpu.make_async_copy(src, dst, sem.at[s])

    cp_fd = copy(fd_hbm, fd_ref, 0)
    x_cols = ((0, 512), (512, 512), (1024, 1024))
    cp_x = [copy(xat_hbm.at[:, pl.ds(o, n)], xat_ref.at[:, pl.ds(o, n)], 40 + i)
            for i, (o, n) in enumerate(x_cols)]
    cp_p0 = pair_copies(0, 0)
    cp_p1 = pair_copies(1, 1)
    cp_c = [[copy(c_hbm.at[pl.ds(o + 512 * i, 512)], c_ref.at[pl.ds(o + 512 * i, 512)], 44 + 2 * i + k)
             for k, o in enumerate((0, S // 2))] for i in range(2)]
    cp_wr = copy(wrt_hbm, wt_ref.at[0], 2)
    cp_wi = copy(wit_hbm, wt_ref.at[1], 3)
    cp_gf = copy(gf_hbm, gf_ref, 4)
    cp_gi = copy(gi_hbm, gi_ref, 5)
    cp_fi = copy(fi_hbm, fi_ref, 6)
    cp_xb = copy(xbt_hbm, xbt_ref, 7)
    for cp in ([cp_fd] + cp_x + cp_p0[:2] + cp_c[0] + [cp_wr, cp_wi, cp_gf, cp_gi]
               + cp_c[1] + [cp_fi, cp_xb, cp_p0[2]] + cp_p1):
        cp.start()

    def proj(i, w, slot):
        _kv_chunk(i, c_ref, ca_ref, wkv_ref.at[w], k_ref.at[slot], v_ref.at[slot])
        _q_chunk(i, xb_ref, wqh_ref.at[w], q_ref.at[slot])

    def relayout(i, unp, slot, w):
        _relayout_piece(i, unp, rawk.at[slot], rawv.at[slot], rawq.at[slot], wkv_ref.at[w], wqh_ref.at[w])

    def kv0(i):
        _kv_chunk(i, c_ref, ca_ref, wkv_ref.at[0], k_ref.at[0], v_ref.at[0])
    cp_fd.wait()
    cp_x[0].wait()

    def a1(ii):
        @pl.when(ii == 1)
        def _():
            cp_x[1].wait()

        @pl.when(ii == 2)
        def _():
            cp_x[2].wait()

        _a_feature_dft(2 * ii, xat_ref, fd_ref, y_ref)
        _a_feature_dft(2 * ii + 1, xat_ref, fd_ref, y_ref)

    _loop(4, a1)
    for cp in cp_p0[:2] + cp_c[0]:
        cp.wait()
    for j in range(8):
        _relayout_piece(j, _lo, rawk.at[0], rawv.at[0], None, wkv_ref.at[0], None)

    def kv_dft(base, sign):
        def body(i):
            _strassen_lhs(base + i, c_ref, ca_ref)
            kv0(base + i)
            _a_dft16(2 * i, sign, y_ref, t_ref)
            _a_dft16(2 * i + 1, sign, y_ref, t_ref)
        return body

    _loop(4, kv_dft(0, -1))
    for cp in (cp_wr, cp_wi, cp_gf):
        cp.wait()
    for a in range(16):
        _a_w_transpose(a, wt_ref, wn_ref)
    for q in range(16):
        _a_fwd_gate(q, gf_ref, t_ref, wn_ref, z_ref)
    for cp in [cp_gi] + cp_c[1]:
        cp.wait()
    for q in range(16):
        _a_inv(q, gi_ref, z_ref, y_ref)
        if q % 2:
            _relayout_piece(q // 2, _hi, rawk.at[0], rawv.at[0], None, wkv_ref.at[1], None)
    _loop(4, kv_dft(4, 1))
    for cp in (cp_fi, cp_xb, cp_p0[2]):
        cp.wait()

    def a5(i):
        for a in range(4):
            _a_feature_idft(4 * i + a, t_ref, fi_ref, y_out_ref)
        _x_lhs(i, xbt_ref, xb_ref)

    _loop(4, a5)
    for j in range(7):
        _relayout_q(j, _lo, rawq.at[0], wqh_ref.at[0])
        _relayout_q(j, _hi, rawq.at[0], wqh_ref.at[1])
    for i in range(8):
        _q_chunk(i, xb_ref, wqh_ref.at[0], q_ref.at[0])

    cp_y = pltpu.make_async_copy(y_out_ref.at[:, pl.ds(0, 384)], out_hbm.at[:, pl.ds(0, 384)], osem.at[0])
    cp_y.start()

    cp_wo = [pltpu.make_async_copy(wot_hbm.at[h], wot_ref.at[:, pl.ds(D * h, D)], sem.at[22 + h])
             for h in range(H)]

    def head_body(h, carry):
        cur = jax.lax.rem(h, 2)
        nxt = 1 - cur
        p = h // 2 + 1
        rslot = jax.lax.rem(p, 2)

        @pl.when(jnp.logical_and(cur == 0, p < H // 2))
        def _():
            for cp in pair_copies(p, rslot):
                cp.wait()

            @pl.when(p + 1 < H // 2)
            def _():
                for cp in pair_copies(p + 1, 1 - rslot):
                    cp.start()

        @pl.when(h == 1)
        def _():
            for cp in cp_wo:
                cp.start()

        @pl.when(h == 4)
        def _():
            for cp in cp_wo:
                cp.wait()
            _out_lhs(wot_ref, wa_ref)

        sh = (16 * nxt).astype(U32)

        def unp(u):
            return pltpu.bitcast((u << sh) & jnp.uint32(0xFFFF0000), F32)

        def fill(i):
            proj(i, nxt, nxt)
            relayout(i, unp, rslot, cur)

        _attn_head(q_ref.at[cur], k_ref.at[cur], v_ref.at[cur], ctx_ref, h, fill)
        return carry
    jax.lax.fori_loop(0, H - 1, head_body, 0)

    def out_copy(i):
        rows = _ds(BQ * i, BQ)
        return pltpu.make_async_copy(y_out_ref.at[rows, :], out_hbm.at[rows, pl.ds(384, 512)], osem.at[1 + i])

    def out_proj(i):
        _out_block(i, ctx_ref, wot_ref, wa_ref, cb_ref, y_out_ref, y_out_ref)
        out_copy(i).start()

    cp_y.wait()

    _attn_head(q_ref.at[1], k_ref.at[1], v_ref.at[1], ctx_ref, H - 1, out_proj, 'q7 q6 p7 q5 f7 p6 q4 f6 p5 q3 f5 p4 q2 f4 p3 q1 f3 p2 q0 p1 f2 p0 f1 f0')
    for i in range(S // BQ):
        out_copy(i).wait()


def _run(A_x, A_w_r, A_w_i, B_x, B_c_kv, B_w_q, B_w_uk, B_w_uv, B_w_o):
    fd, gf, gi, fi = _dft_constants()
    any_spec = pl.BlockSpec(memory_space=pl.ANY)
    out = pl.pallas_call(
        _kernel,
        out_shape=jax.ShapeDtypeStruct((S, 2 * DM), BF16),
        in_specs=[any_spec] * 13,
        out_specs=any_spec,
        scratch_shapes=[
            pltpu.VMEM((DM, S), BF16),
            pltpu.VMEM((2, DF, S), BF16),
            pltpu.VMEM((DM, 512), BF16),
            pltpu.VMEM((16, 256, 128), BF16),
            pltpu.VMEM((16, 256, 128), BF16),
            pltpu.VMEM((512, 512), BF16),
            pltpu.VMEM((S, 512), F32),
            pltpu.VMEM((16, 128, 512), BF16),
            pltpu.VMEM((16, 128, 512), BF16),
            pltpu.VMEM((4, S, 128), BF16),
            pltpu.VMEM((DM, S), BF16),
            pltpu.VMEM((7, S // 2, DM // 2), BF16),
            pltpu.VMEM((S, DC), BF16),
            pltpu.VMEM((5, S // 2, DC // 2), BF16),
            pltpu.VMEM((2, DC, D), U32),
            pltpu.VMEM((2, DC, D), U32),
            pltpu.VMEM((2, DM, D), U32),
            pltpu.VMEM((2, 7, DC // 2, D), BF16),
            pltpu.VMEM((2, 7, DM // 2, D // 2), BF16),
            pltpu.VMEM((2, S, D), BF16),
            pltpu.VMEM((2, S, D), BF16),
            pltpu.VMEM((2, S, D), BF16),
            pltpu.VMEM((S, H * D), BF16),
            pltpu.VMEM((DM, H * D), BF16),
            pltpu.VMEM((5, DM // 2, H * D // 2), BF16),
            pltpu.VMEM((5, 128, H * D // 2), BF16),
            pltpu.VMEM((S, 512), BF16),
            pltpu.SemaphoreType.DMA((56,)),
            pltpu.SemaphoreType.DMA((16,)),
        ],
        compiler_params=pltpu.CompilerParams(vmem_limit_bytes=110 * 1024 * 1024),
    )(A_x[0].T, A_w_r.T, A_w_i.T, B_x[0].T, B_c_kv[0], B_w_q, B_w_uk, B_w_uv,
      jnp.swapaxes(B_w_o, 1, 2), fd, gf, gi, fi)
    return out[None]


@jax.jit
def pallas_concat_heads__spectral_gfnet__compressed_kv_cla__prompt_kernel(
    A_x: jax.Array,
    A_w_r: jax.Array,
    A_w_i: jax.Array,
    B_x: jax.Array,
    B_c_kv: jax.Array,
    B_w_q: jax.Array,
    B_w_uk: jax.Array,
    B_w_uv: jax.Array,
    B_w_o: jax.Array,
):
    return _run(A_x, A_w_r, A_w_i, B_x, B_c_kv, B_w_q, B_w_uk, B_w_uv, B_w_o)
```
